```python
import jax
import jax.numpy as jnp

def _softmax(x, axis=-1):
    return jax.nn.softmax(x, axis=axis)
def _gelu(x):
    return jax.nn.gelu(x, approximate=True)
def _silu(x):
    return jax.nn.silu(x)
def _sigmoid(x):
    return jax.nn.sigmoid(x)
def _layernorm(x, axis=-1, eps=1e-5):
    m = jnp.mean(x, axis=axis, keepdims=True)
    v = jnp.var(x, axis=axis, keepdims=True)
    return (x - m) / jnp.sqrt(v + eps)
def _scatter_add(tgt, idx, src, axis=0):
    return tgt.at[idx].add(src)
def _segment_sum(src, seg, n):
    return jax.ops.segment_sum(src, seg, n)
class _Rng:
    def __init__(self, key):
        self._k = key
    def _next(self):
        self._k, sub = jax.random.split(self._k)
        return sub
    def normal(self, shape):
        return jax.random.normal(self._next(), shape, dtype=jnp.bfloat16)
    def randint(self, lo, hi, shape):
        return jax.random.randint(self._next(), shape, lo, hi, dtype=jnp.int32)
    def uniform(self, shape, lo=0.0, hi=1.0):
        return jax.random.uniform(self._next(), shape, jnp.bfloat16, lo, hi)
    def permutation(self, n):
        return jax.random.permutation(self._next(), n)


kernel_name = 'interleave_layers__linear_kernel_hedgehog__sliding_local_dilated__prompt'

def setup_inputs():
    _rng = _Rng(jax.random.key(int.from_bytes(__import__("os").urandom(4), "little")))
    _w = (lambda a: (lambda t: t.astype(jnp.bfloat16) if jnp.issubdtype(t.dtype, jnp.floating) else t)(jnp.asarray(a)))
    def _A_setup():
        B, S, D, H = 1, 2048, 1024, 32
        Dh = D // H
        return {
            "x": _w((lambda *s: _rng.normal(s) * 0.05)(B, S, D)),
            "wqkv": _w((lambda *s: _rng.normal(s) * 0.05)(D, 3 * D)),
            "w_phi": _w((lambda *s: _rng.normal(s) * 0.05)(H, Dh, Dh) * (Dh ** -0.5)),
            "wo": _w((lambda *s: _rng.normal(s) * 0.05)(D, D)),
        }
    _A_in = _A_setup()

    def _B_setup():
        B, S, D = 1, 2048, 1024
        return {
            "x": _w((lambda *s: _rng.normal(s) * 0.05)(B, S, D)),
            "wqkv": _w((lambda *s: _rng.normal(s) * 0.05)(D, 3 * D)),
            "wo": _w((lambda *s: _rng.normal(s) * 0.05)(D, D)),
        }
    _B_in = _B_setup()

    return {
        "A_x": _A_in["x"],
        "A_wqkv": _A_in["wqkv"],
        "A_w_phi": _A_in["w_phi"],
        "A_wo": _A_in["wo"],
        "B_x": _B_in["x"],
        "B_wqkv": _B_in["wqkv"],
        "B_wo": _B_in["wo"],
    }

def reference(A_x, A_wqkv, A_w_phi, A_wo, B_x, B_wqkv, B_wo):
    def _A_ref(x, wqkv, w_phi, wo):
        B, S, D = x.shape
        H = 32; Dh = D // H
        qkv = (lambda x, *d: x.transpose(*d))((x @ wqkv).reshape(B, S, 3, H, Dh), 2, 0, 3, 1, 4)
        q, k, v = qkv[0], qkv[1], qkv[2]
        pq = jnp.einsum("bhsd,hdf->bhsf", q, w_phi)
        pk = jnp.einsum("bhsd,hdf->bhsf", k, w_phi)
        phi_q = jnp.concatenate([_softmax(pq, axis=-1), _softmax(-pq, axis=-1)], axis=-1)
        phi_k = jnp.concatenate([_softmax(pk, axis=-1), _softmax(-pk, axis=-1)], axis=-1)
        kv = jnp.einsum("bhsf,bhsd->bhfd", phi_k, v)
        z  = jnp.einsum("bhsf->bhf", phi_k)
        num = jnp.einsum("bhqf,bhfd->bhqd", phi_q, kv)
        den = jnp.einsum("bhqf,bhf->bhq", phi_q, z)[..., None] + 1e-6
        o = num / den
        return (lambda x, *d: x.transpose(*d))(o, 0, 2, 1, 3).reshape(B, S, D) @ wo

    def _B_ref(x, wqkv, wo):
        B, S, D = x.shape
        H = 32; Dh = D // H
        W, dil = 8, 2
        qkv = (lambda x, *d: x.transpose(*d))((x @ wqkv).reshape(B, S, 3, H, Dh), 2, 0, 3, 1, 4)
        q, k, v = qkv[0], qkv[1], qkv[2]
        scale = Dh ** -0.5
        pos = jnp.arange(S)
        off = jnp.arange(W) * dil
        idx = pos[:, None] - off[None, :]
        mask = idx >= 0
        idx_c = jnp.where(mask, idx, 0).reshape(-1)
        kg = k[:, :, idx_c, :].reshape(B, H, S, W, Dh)
        vg = v[:, :, idx_c, :].reshape(B, H, S, W, Dh)
        logits = jnp.einsum("bhsd,bhswd->bhsw", q, kg) * scale
        logits = jnp.where(mask[None, None, :, :], logits, -1e9)
        attn = _softmax(logits, axis=-1)
        o = jnp.einsum("bhsw,bhswd->bhsd", attn, vg)
        return (lambda x, *d: x.transpose(*d))(o, 0, 2, 1, 3).reshape(B, S, D) @ wo

    x = A_x
    x = x + _A_ref(_layernorm(x, axis=-1), A_wqkv, A_w_phi, A_wo)
    x = x + _B_ref(_layernorm(x, axis=-1), B_wqkv, B_wo)
    x = x + _A_ref(_layernorm(x, axis=-1), A_wqkv, A_w_phi, A_wo)
    x = x + _B_ref(_layernorm(x, axis=-1), B_wqkv, B_wo)
    return x
```

```python
import jax
import jax.numpy as jnp
import jax.experimental.pallas as pl
import jax.experimental.pallas.tpu as pltpu

f32 = jnp.float32
bf16 = jnp.bfloat16
u32 = jnp.uint32

S, D, H, DH = 2048, 1024, 32, 32
NG = 8
NJ = 16
W, DIL = 8, 2
SCALE = float(DH) ** -0.5
NT = (((1,), (1,)), ((), ()))


NN = (((1,), (0,)), ((), ()))


def _mm(a, b, dims=NN):
    return jax.lax.dot_general(a, b, dims, preferred_element_type=f32)


def _recip(x):
    r = pl.reciprocal(x, approx=True)
    return r * (2.0 - x * r)


def _phi(p):
    p3 = p.reshape(4, 32, 128)
    mx = jnp.max(p3, axis=1, keepdims=True)
    mn = jnp.min(p3, axis=1, keepdims=True)
    e1 = jnp.exp(p3 - mx)
    e2 = jnp.exp(mn - p3)
    s1 = jnp.sum(e1, axis=1, keepdims=True)
    s2 = jnp.sum(e2, axis=1, keepdims=True)
    a = (e1 * _recip(s1)).reshape(128, 128).astype(bf16)
    b = (e2 * _recip(s2)).reshape(128, 128).astype(bf16)
    t0 = jnp.concatenate([a[0:64], b[0:64]], axis=0)
    t1 = jnp.concatenate([a[64:128], b[64:128]], axis=0)
    return t0, t1


def _kernel(x_ref, awqkv_ref, awphi_ref, awo_ref, bwqkv_ref, bwo_ref, out_ref,
            xT, lnT, WA, WoA, WB, WoB, pbuf, lhsA, stage):

    def jsl(j):
        return slice(j * 128, (j + 1) * 128)

    for r in range(16):
        for c in range(8):
            blk = x_ref[r * 128:(r + 1) * 128, c * 128:(c + 1) * 128]
            stage[c, r * 64:(r + 1) * 64, :] = pltpu.bitcast(blk, u32)
    for i in range(8):
        for c in range(8):
            wd = stage.at[c][pl.ds(i, 128, stride=8), :].T
            lo = pltpu.bitcast(wd << 16, f32)
            hi = pltpu.bitcast(wd & jnp.uint32(0xFFFF0000), f32)
            xT[c * 128:(c + 1) * 128, jsl(2 * i)] = lo
            xT[c * 128:(c + 1) * 128, jsl(2 * i + 1)] = hi

    f_i = jax.lax.broadcasted_iota(jnp.int32, (32, 128), 0)
    c_i = jax.lax.broadcasted_iota(jnp.int32, (32, 128), 1)
    R = jnp.where(c_i % 32 == f_i, 1.0, 0.0).astype(bf16)
    r2 = jax.lax.broadcasted_iota(jnp.int32, (128, 128), 0)
    c2 = jax.lax.broadcasted_iota(jnp.int32, (128, 128), 1)
    blockmask = (r2 // 32) == (c2 // 32)
    for g in range(NG):
        Bm = awphi_ref[4 * g:4 * g + 4].reshape(128, 32)
        Phi = jnp.where(blockmask, _mm(Bm, R), 0.0)
        PhiT = Phi.T.astype(bf16)
        for part in range(2):
            blk = awqkv_ref[:, part * D + g * 128: part * D + (g + 1) * 128]
            r = _mm(PhiT, blk, NT)
            WA[g, part * 128:(part + 1) * 128, :] = r.astype(bf16)
        WA[g, 256:384, :] = awqkv_ref[:, 2 * D + g * 128: 2 * D + (g + 1) * 128].T
        WoA[g] = awo_ref[g * 128:(g + 1) * 128, :].T
        for part in range(3):
            WB[g, part * 128:(part + 1) * 128, :] = bwqkv_ref[:, part * D + g * 128: part * D + (g + 1) * 128].T
        WoB[g] = bwo_ref[g * 128:(g + 1) * 128, :].T

    lane = jax.lax.broadcasted_iota(jnp.int32, (4, 1, 128), 2)
    lane0 = lane == 0
    ones16 = jnp.ones((16, 128), bf16)

    def ln_step(j):
        x = xT[:, jsl(j)]
        m = jnp.sum(x, axis=0, keepdims=True) * (1.0 / D)
        xc = x - m
        v = jnp.sum(xc * xc, axis=0, keepdims=True) * (1.0 / D)
        lnT[:, jsl(j)] = (xc * jax.lax.rsqrt(v + 1e-5)).astype(bf16)

    def proj(Wref, g, j):
        return _mm(Wref[g], lnT[:, jsl(j)])

    def out_proj(Woref, g, j, o):
        xT[:, jsl(j)] += _mm(Woref[g], o)

    def kv_step(pk, v, acc):
        t0, t1 = _phi(pk)
        vb = v.astype(bf16)
        l0 = jnp.concatenate([vb[0:64], ones16], axis=0)
        l1 = jnp.concatenate([vb[64:128], ones16], axis=0)
        a0 = _mm(l0, t0, NT)
        a1 = _mm(l1, t1, NT)
        if acc is None:
            return a0, a1
        return acc[0] + a0, acc[1] + a1

    rr = jax.lax.broadcasted_iota(jnp.int32, (80, 128), 0)
    cc = jax.lax.broadcasted_iota(jnp.int32, (80, 128), 1)
    row_head = jnp.where(rr < 64, rr // 32, (rr - 64) // 8)
    kvmask = row_head == ((cc // 32) % 2)

    def kv_final(acc, slot):
        lhsA[slot, 0] = jnp.where(kvmask, acc[0], 0.0).astype(bf16)
        lhsA[slot, 1] = jnp.where(kvmask, acc[1], 0.0).astype(bf16)

    def num_step(pq, slot):
        t0, t1 = _phi(pq)
        outs = []
        for p, t in ((0, t0), (1, t1)):
            r = _mm(lhsA[slot, p], t)
            for hh in range(2):
                den = r[64 + 8 * hh: 72 + 8 * hh] + 1e-6
                num = r[32 * hh: 32 * hh + 32].reshape(4, 8, 128)
                outs.append((num * _recip(den)[None]).reshape(32, 128))
        return jnp.concatenate(outs, axis=0).astype(bf16)

    def att_tile(slot, j, kcache, vcache):
        def get(cache, base, jj):
            if jj not in cache:
                if jj >= 0:
                    cache[jj] = pbuf[slot, base:base + 128, jsl(jj)]
                else:
                    cache[jj] = pltpu.roll(pbuf[slot, base:base + 128, jsl(jj + 16)], 1, 1)
            return cache[jj]
        q = pbuf[slot, 0:128, jsl(j)]
        ls = []
        for w in range(W):
            jj = j - DIL * w
            kk = get(kcache, 128, jj)
            l = jnp.sum((q * kk).reshape(4, 32, 128), axis=1, keepdims=True) * SCALE
            if jj < 0:
                l = jnp.where(lane0, -1e9, l)
            ls.append(l)
        m = ls[0]
        for w in range(1, W):
            m = jnp.maximum(m, ls[w])
        es = [jnp.exp(l - m) for l in ls]
        ssum = es[0]
        for w in range(1, W):
            ssum = ssum + es[w]
        r = _recip(ssum)
        o = None
        for w in range(W):
            vv = get(vcache, 256, j - DIL * w).reshape(4, 32, 128)
            t = (es[w] * r) * vv
            o = t if o is None else o + t
        return o.reshape(128, 128).astype(bf16)

    def a_front(g, slot, pre=None, post=None):
        acc = None
        pend = None
        for j in range(NJ):
            if pre is not None:
                pre(j)
            r = proj(WA, g, j)
            pbuf[slot, 0:128, jsl(j)] = r[0:128]
            if pend is not None:
                acc = kv_step(pend[0], pend[1], acc)
            pend = (r[128:256], r[256:384])
            if post is not None:
                post(j)
        acc = kv_step(pend[0], pend[1], acc)
        kv_final(acc, slot)

    def a_back_step(g, slot, j):
        o = num_step(pbuf[slot, 0:128, jsl(j)], slot)
        out_proj(WoA, g, j, o)

    def b_front(g, slot, pre=None, post=None):
        for j in range(NJ):
            if pre is not None:
                pre(j)
            pbuf[slot, :, jsl(j)] = proj(WB, g, j)
            if post is not None:
                post(j)

    def b_back(g, slot):
        kc, vc = {}, {}
        def step(j):
            out_proj(WoB, g, j, att_tile(slot, j, kc, vc))
        return step

    def layer_pair(first):
        if first:
            a_front(0, 0, pre=ln_step)
        else:
            st = b_back(NG - 1, 1)
            def pre(j):
                st(j)
                ln_step(j)
            a_front(0, 0, pre=pre)

        def a_body(g, _):
            slot = g % 2
            a_front(g, slot, post=lambda j: a_back_step(g - 1, 1 - slot, j))
            return 0
        jax.lax.fori_loop(1, NG, a_body, 0)

        def pre_b(j):
            a_back_step(NG - 1, (NG - 1) % 2, j)
            ln_step(j)
        b_front(0, 0, pre=pre_b)

        def b_body(g, _):
            slot = g % 2
            b_front(g, slot, post=b_back(g - 1, 1 - slot))
            return 0
        jax.lax.fori_loop(1, NG, b_body, 0)

    layer_pair(True)
    layer_pair(False)
    st = b_back(NG - 1, 1)
    for j in range(NJ):
        st(j)

    for i in range(8):
        for c in range(8):
            lo = xT[c * 128:(c + 1) * 128, jsl(2 * i)]
            hi = xT[c * 128:(c + 1) * 128, jsl(2 * i + 1)]
            lo = pltpu.bitcast(lo.astype(bf16).astype(f32), u32) >> 16
            hi = pltpu.bitcast(hi.astype(bf16).astype(f32), u32)
            wd = lo | hi
            stage.at[c][pl.ds(i, 128, stride=8), :] = wd.T
    for r in range(16):
        for c in range(8):
            out_ref[r * 128:(r + 1) * 128, c * 128:(c + 1) * 128] = pltpu.bitcast(stage[c, r * 64:(r + 1) * 64, :], bf16)


@jax.jit
def pallas_interleave_layers__linear_kernel_hedgehog__sliding_local_dilated__prompt_kernel(
    A_x, A_wqkv, A_w_phi, A_wo, B_x, B_wqkv, B_wo):
    del B_x
    x2 = A_x.reshape(S, D)
    out = pl.pallas_call(
        _kernel,
        out_shape=jax.ShapeDtypeStruct((S, D), bf16),
        scratch_shapes=[
            pltpu.VMEM((D, S), f32),
            pltpu.VMEM((D, S), bf16),
            pltpu.VMEM((NG, 384, D), bf16),
            pltpu.VMEM((NG, D, 128), bf16),
            pltpu.VMEM((NG, 384, D), bf16),
            pltpu.VMEM((NG, D, 128), bf16),
            pltpu.VMEM((2, 384, S), f32),
            pltpu.VMEM((2, 2, 80, 128), bf16),
            pltpu.VMEM((8, S // 2, 128), u32),
        ],
        compiler_params=pltpu.CompilerParams(vmem_limit_bytes=100 * 1024 * 1024),
    )(x2, A_wqkv, A_w_phi, A_wo, B_wqkv, B_wo)
    return out.reshape(1, S, D)
```

```python
import jax
import jax.numpy as jnp
import jax.experimental.pallas as pl
import jax.experimental.pallas.tpu as pltpu

f32 = jnp.float32
bf16 = jnp.bfloat16
u32 = jnp.uint32

S, D, H, DH = 2048, 1024, 32, 32
PART = 'ALL'
CFG = ''
FLAGS = None
WC = int('4')
OSPLIT = int('4')
PSK = int('1')
PORD = int('0')
NG = 8
NJ = 16
W, DIL = 8, 2
SCALE = float(DH) ** -0.5
NT = (((1,), (1,)), ((), ()))


NN = (((1,), (0,)), ((), ()))


def _mm(a, b, dims=NN):
    return jax.lax.dot_general(a, b, dims, preferred_element_type=f32)


def _pk(x):
    return pltpu.bitcast(x, u32)


def _up(x):
    return pltpu.bitcast(x, bf16)


def _recip(x):
    r = pl.reciprocal(x, approx=True)
    return r * (2.0 - x * r)


def _phi(p):
    p3 = p.reshape(4, 32, 128)
    mx = jnp.max(p3, axis=1, keepdims=True)
    mn = jnp.min(p3, axis=1, keepdims=True)
    e1 = jnp.exp(p3 - mx)
    e2 = jnp.exp(mn - p3)
    s1 = jnp.sum(e1, axis=1, keepdims=True)
    s2 = jnp.sum(e2, axis=1, keepdims=True)
    a = (e1 * _recip(s1)).reshape(128, 128)
    b = (e2 * _recip(s2)).reshape(128, 128)
    t0 = jnp.concatenate([a[0:64], b[0:64]], axis=0).astype(bf16)
    t1 = jnp.concatenate([a[64:128], b[64:128]], axis=0).astype(bf16)
    return t0, t1


def _kernel(x_ref, awqkv_ref, awphi_ref, awo_ref, bwqkv_ref, bwo_ref, out_ref,
            xT, lnT, WA, WoA, WB, WoB, pbuf, lhsA, stage):

    def jsl(j):
        return slice(j * 128, (j + 1) * 128)

    for r in range(16 if PART == 'ALL' else 0):
        for c in range(8):
            blk = x_ref[r * 128:(r + 1) * 128, c * 128:(c + 1) * 128]
            stage[c, r * 64:(r + 1) * 64, :] = pltpu.bitcast(blk, u32)
    for i in range(8 if PART == 'ALL' else 0):
        for c in range(8):
            wd = stage.at[c][pl.ds(i, 128, stride=8), :].T
            lo = pltpu.bitcast(wd << 16, f32)
            hi = pltpu.bitcast(wd & jnp.uint32(0xFFFF0000), f32)
            xT[2 * i, c * 128:(c + 1) * 128, :] = lo
            xT[2 * i + 1, c * 128:(c + 1) * 128, :] = hi

    f_i = jax.lax.broadcasted_iota(jnp.int32, (32, 128), 0)
    c_i = jax.lax.broadcasted_iota(jnp.int32, (32, 128), 1)
    R = jnp.where(c_i % 32 == f_i, 1.0, 0.0).astype(bf16)
    r2 = jax.lax.broadcasted_iota(jnp.int32, (128, 128), 0)
    c2 = jax.lax.broadcasted_iota(jnp.int32, (128, 128), 1)
    blockmask = (r2 // 32) == (c2 // 32)
    for g in range(NG if PART == 'ALL' else 0):
        Bm = awphi_ref[4 * g:4 * g + 4].reshape(128, 32)
        Phi = jnp.where(blockmask, _mm(Bm, R), 0.0)
        PhiT = Phi.T.astype(bf16)
        for part in range(2):
            blk = awqkv_ref[:, part * D + g * 128: part * D + (g + 1) * 128]
            r = _mm(PhiT, blk, NT)
            for k in range(8):
                WA[g, k, part * 64:(part + 1) * 64, :] = _pk(r[:, k * 128:(k + 1) * 128].astype(bf16))
        for k in range(8):
            WA[g, k, 128:192, :] = _pk(awqkv_ref[k * 128:(k + 1) * 128, 2 * D + g * 128: 2 * D + (g + 1) * 128].T)
        WoA[g] = _pk(awo_ref[g * 128:(g + 1) * 128, :].T)
        for part in range(3):
            for k in range(8):
                WB[g, k, part * 64:(part + 1) * 64, :] = _pk(bwqkv_ref[k * 128:(k + 1) * 128, part * D + g * 128: part * D + (g + 1) * 128].T)
        WoB[g] = _pk(bwo_ref[g * 128:(g + 1) * 128, :].T)

    lane = jax.lax.broadcasted_iota(jnp.int32, (4, 1, 128), 2)
    lane0 = lane == 0
    ones16 = jnp.ones((16, 128), f32)

    def ln_step(j):
        x = xT[j]
        m = jnp.sum(x, axis=0, keepdims=True) * (1.0 / D)
        xc = x - m
        v = jnp.sum(xc * xc, axis=0, keepdims=True) * (1.0 / D)
        lnT[j] = (xc * jax.lax.rsqrt(v + 1e-5)).astype(bf16)

    def proj(Wref, g, j):
        return _mm(jnp.concatenate([_up(Wref[g, k]) for k in range(8)], axis=1), lnT[j])

    def out_proj(Woref, g, j, o):
        n = 1024 // OSPLIT
        for q in range(OSPLIT):
            xT[j, q * n:(q + 1) * n, :] += _mm(_up(Woref[g, q * n // 2:(q + 1) * n // 2, :]), o)

    def kv_step(pk, v, acc):
        t0, t1 = _phi(pk)
        l0 = jnp.concatenate([v[0:64], ones16], axis=0).astype(bf16)
        l1 = jnp.concatenate([v[64:128], ones16], axis=0).astype(bf16)
        a0 = _mm(l0, t0, NT)
        a1 = _mm(l1, t1, NT)
        if acc is None:
            return a0, a1
        return acc[0] + a0, acc[1] + a1

    rr = jax.lax.broadcasted_iota(jnp.int32, (80, 128), 0)
    cc = jax.lax.broadcasted_iota(jnp.int32, (80, 128), 1)
    row_head = jnp.where(rr < 64, rr // 32, (rr - 64) // 8)
    kvmask = row_head == ((cc // 32) % 2)

    def kv_final(acc, slot):
        lhsA[slot, 0] = _pk(jnp.where(kvmask, acc[0], 0.0).astype(bf16))
        lhsA[slot, 1] = _pk(jnp.where(kvmask, acc[1], 0.0).astype(bf16))

    def num_step(pq, slot):
        t0, t1 = _phi(pq)
        outs = []
        for p, t in ((0, t0), (1, t1)):
            r = _mm(_up(lhsA[slot, p]), t)
            for hh in range(2):
                den = r[64 + 8 * hh: 72 + 8 * hh] + 1e-6
                num = r[32 * hh: 32 * hh + 32].reshape(4, 8, 128)
                outs.append((num * _recip(den)[None]).reshape(32, 128))
        return jnp.concatenate(outs, axis=0).astype(bf16)

    def att_tile(slot, j, kcache, vcache):
        def get(cache, base, jj):
            if jj not in cache:
                if jj >= 0:
                    cache[jj] = pbuf[slot, jj, base:base + 128, :]
                else:
                    cache[jj] = pltpu.roll(pbuf[slot, jj + 16, base:base + 128, :], 1, 1)
            return cache[jj]
        def one(h0, nh, dep):
            rows = lambda base: slice(base + 32 * h0, base + 32 * (h0 + nh))
            q = pbuf[slot, j, rows(0), :].reshape(nh, 32, 128)
            if dep is not None:
                q = q + dep
            ls = []
            for w in range(W):
                jj = j - DIL * w
                kk = get(kcache, 128, jj)[32 * h0: 32 * (h0 + nh)].reshape(nh, 32, 128)
                if 'wchain' in CFG and w > 0 and w % WC == 0:
                    qq = q + ls[-1][0:1] * 0.0
                else:
                    qq = q
                l = jnp.sum(qq * kk, axis=1, keepdims=True) * SCALE
                if jj < 0:
                    l = jnp.where(lane0[:nh], -1e9, l)
                ls.append(l)
            m = ls[0]
            for w in range(1, W):
                m = jnp.maximum(m, ls[w])
            es = [jnp.exp(l - m) for l in ls]
            ssum = es[0]
            for w in range(1, W):
                ssum = ssum + es[w]
            r = _recip(ssum)
            o = None
            for w in range(W):
                vv = get(vcache, 256, j - DIL * w)[32 * h0: 32 * (h0 + nh)].reshape(nh, 32, 128)
                t = (es[w] * r) * vv
                o = t if o is None else o + t
            return o
        if 'chain' in CFG:
            nh = 2 if 'chain2' in CFG else 1
            outs = []
            dep = None
            for h0 in range(0, 4, nh):
                o = one(h0, nh, dep)
                dep = o[0:1, 0:1, :] * 0.0
                outs.append(o.reshape(32 * nh, 128))
            return jnp.concatenate(outs, axis=0).astype(bf16)
        return one(0, 4, None).reshape(128, 128).astype(bf16)

    def block(front, back, ln):
        st = {'acc': None}
        pend, ots = {}, {}
        kc, vc = {}, {}
        ft = front[0] if front else None
        bt = back[0] if back else None
        order = list(range(NJ - 1, -1, -1)) if bt == 'B' else list(range(NJ))

        def P(j):
            _, g, slot = front
            if ln:
                ln_step(j)
            r = proj(WA if ft == 'A' else WB, g, j)
            if ft == 'A':
                pbuf[slot, j, 0:128, :] = r[0:128]
                pend[j] = (r[128:256], r[256:384])
            else:
                pbuf[slot, j] = r

        def KV(j):
            pk, v = pend.pop(j)
            st['acc'] = kv_step(pk, v, st['acc'])

        def NUM(j):
            _, g, slot = back
            ots[j] = num_step(pbuf[slot, j, 0:128, :], slot)

        def O(j):
            _, g, slot = back
            if bt == 'A':
                out_proj(WoA, g, j, ots.pop(j))
            else:
                out_proj(WoB, g, j, att_tile(slot, j, kc, vc))

        psk = PSK if (ln and back) else 0
        for t in range(-1, NJ + psk + 2):
            if bt == 'A' and 0 <= t + 1 < NJ:
                NUM(order[t + 1])
            if psk and 0 <= t < NJ:
                O(order[t])
            if front and 0 <= t - psk < NJ:
                P((order if ln or PORD else list(range(NJ)))[t - psk])
            if not psk and back and 0 <= t < NJ:
                O(order[t])
            if ft == 'A' and 0 <= t - psk - 1 < NJ:
                KV(order[t - psk - 1])
        if ft == 'A':
            kv_final(st['acc'], front[2])

    def a_loop():
        def body(g, _):
            slot = g % 2
            block(('A', g, slot), ('A', g - 1, 1 - slot), False)
            return 0
        jax.lax.fori_loop(1, NG, body, 0)

    def b_loop():
        def body(g, _):
            slot = g % 2
            block(('B', g, slot), ('B', g - 1, 1 - slot), False)
            return 0
        jax.lax.fori_loop(1, NG, body, 0)

    L = (NG - 1) % 2
    if PART == 'A':
        a_loop()
    elif PART == 'B':
        b_loop()
    elif PART == 'BS':
        block(('B', 1, 0), ('B', 0, 1), False)
    elif PART == 'AS':
        block(('A', 1, 0), ('A', 0, 1), False)
    elif PART == 'AB':
        block(('B', 0, 0), ('A', NG - 1, L), True)
    elif PART == 'BA':
        block(('A', 0, 0), ('B', NG - 1, L), True)
    elif PART == 'INIT':
        block(('A', 0, 0), None, True)
    elif PART == 'FIN':
        block(None, ('B', NG - 1, L), False)
    else:
        block(('A', 0, 0), None, True)
        a_loop()
        block(('B', 0, 0), ('A', NG - 1, L), True)
        b_loop()
        block(('A', 0, 0), ('B', NG - 1, L), True)
        a_loop()
        block(('B', 0, 0), ('A', NG - 1, L), True)
        b_loop()
        block(None, ('B', NG - 1, L), False)

    if PART != 'ALL':
        acc = jnp.zeros((128, 128), f32)
        for j in range(NJ):
            acc = acc + xT[j, 0:128, :] + xT[j, 896:1024, :] + pbuf[0, j, 0:128, :] + pltpu.bitcast(lhsA[0, 0, 0:8, :], f32)[0:1]
        out_ref[0:128, 0:128] = acc.astype(bf16)
        return
    for i in range(8):
        for c in range(8):
            lo = xT[2 * i, c * 128:(c + 1) * 128, :]
            hi = xT[2 * i + 1, c * 128:(c + 1) * 128, :]
            lo = pltpu.bitcast(lo.astype(bf16).astype(f32), u32) >> 16
            hi = pltpu.bitcast(hi.astype(bf16).astype(f32), u32)
            wd = lo | hi
            stage.at[c][pl.ds(i, 128, stride=8), :] = wd.T
    for r in range(16):
        for c in range(8):
            out_ref[r * 128:(r + 1) * 128, c * 128:(c + 1) * 128] = pltpu.bitcast(stage[c, r * 64:(r + 1) * 64, :], bf16)


@jax.jit
def pallas_interleave_layers__linear_kernel_hedgehog__sliding_local_dilated__prompt_kernel(
    A_x, A_wqkv, A_w_phi, A_wo, B_x, B_wqkv, B_wo):
    del B_x
    x2 = A_x.reshape(S, D)
    out = pl.pallas_call(
        _kernel,
        out_shape=jax.ShapeDtypeStruct((S, D), bf16),
        scratch_shapes=[
            pltpu.VMEM((NJ, D, 128), f32),
            pltpu.VMEM((NJ, D, 128), bf16),
            pltpu.VMEM((NG, 8, 192, 128), u32),
            pltpu.VMEM((NG, D // 2, 128), u32),
            pltpu.VMEM((NG, 8, 192, 128), u32),
            pltpu.VMEM((NG, D // 2, 128), u32),
            pltpu.VMEM((2, NJ, 384, 128), f32),
            pltpu.VMEM((2, 2, 40, 128), u32),
            pltpu.VMEM((8, S // 2, 128), u32),
        ],
        compiler_params=pltpu.CompilerParams(vmem_limit_bytes=100 * 1024 * 1024, flags=FLAGS),
    )(x2, A_wqkv, A_w_phi, A_wo, B_wqkv, B_wo)
    return out.reshape(1, S, D)
```

```python
import jax
import jax.numpy as jnp
import jax.experimental.pallas as pl
import jax.experimental.pallas.tpu as pltpu

f32 = jnp.float32
bf16 = jnp.bfloat16
u32 = jnp.uint32

S, D, H, DH = 2048, 1024, 32, 32
PART = 'ALL'
CFG = ''
FLAGS = None
WC = int('4')
OSPLIT = int('4')
PSK = int('1')
PORD = int('0')
PREPPOS = int('9')
PP = 'ft'
INJ = int('0')
NG = 8
NJ = 16
W, DIL = 8, 2
SCALE = float(DH) ** -0.5
NT = (((1,), (1,)), ((), ()))


NN = (((1,), (0,)), ((), ()))


def _mm(a, b, dims=NN):
    return jax.lax.dot_general(a, b, dims, preferred_element_type=f32)


WBF = '0' == '1'
PW = 1 if WBF else 2


def _pw(x):
    return x if WBF else pltpu.bitcast(x, u32)


def _uw(x):
    return x if WBF else pltpu.bitcast(x, bf16)


def _pk(x):
    return pltpu.bitcast(x, u32)


def _up(x):
    return pltpu.bitcast(x, bf16)


def _recip(x):
    r = pl.reciprocal(x, approx=True)
    return r * (2.0 - x * r)


def _phi(p):
    p3 = p.reshape(4, 32, 128)
    mx = jnp.max(p3, axis=1, keepdims=True)
    mn = jnp.min(p3, axis=1, keepdims=True)
    e1 = jnp.exp(p3 - mx)
    e2 = jnp.exp(mn - p3)
    s1 = jnp.sum(e1, axis=1, keepdims=True)
    s2 = jnp.sum(e2, axis=1, keepdims=True)
    a = (e1 * _recip(s1)).reshape(128, 128)
    b = (e2 * _recip(s2)).reshape(128, 128)
    t0 = jnp.concatenate([a[0:64], b[0:64]], axis=0).astype(bf16)
    t1 = jnp.concatenate([a[64:128], b[64:128]], axis=0).astype(bf16)
    return t0, t1


def _kernel(x_hbm, awqkv_hbm, awphi_ref, awo_hbm, bwqkv_hbm, bwo_hbm, out_hbm,
            xT, lnT, WW, WO, pbuf, lhsA, stage, xraw, wraw, oraw, zref, sems):
    zref[...] = jnp.zeros((8, 128), u32)
    full = PART == 'ALL'

    def x_copy(c):
        return pltpu.make_async_copy(x_hbm.at[:, pl.ds(c * 128, 128)], xraw.at[c], sems.at[0, c])

    def col(hbm, part, g):
        return hbm.at[:, pl.ds(pl.multiple_of(part * D + g * 128, 128), 128)]

    def wa_copies(g):
        return [pltpu.make_async_copy(col(awqkv_hbm, p, g), wraw.at[g, p], sems.at[1 + p, g]) for p in range(3)]

    def wb_copies(g):
        return [pltpu.make_async_copy(col(bwqkv_hbm, p, g), wraw.at[g, 4 + p], sems.at[5 + p, g]) for p in range(3)]

    def wo_copies(g):
        rows = pl.ds(pl.multiple_of(g * 128, 128), 128)
        return [pltpu.make_async_copy(awo_hbm.at[rows, :], oraw.at[0, g], sems.at[4, g]),
                pltpu.make_async_copy(bwo_hbm.at[rows, :], oraw.at[1, g], sems.at[8, g])]

    def rest_copies(g):
        return wo_copies(g) + wb_copies(g)

    f_i = jax.lax.broadcasted_iota(jnp.int32, (32, 128), 0)
    c_i = jax.lax.broadcasted_iota(jnp.int32, (32, 128), 1)
    R = jnp.where(c_i % 32 == f_i, 1.0, 0.0).astype(bf16)
    r2 = jax.lax.broadcasted_iota(jnp.int32, (128, 128), 0)
    c2 = jax.lax.broadcasted_iota(jnp.int32, (128, 128), 1)
    blockmask = (r2 // 32) == (c2 // 32)

    def prep_wa_pieces(g):
        memo = {}

        def phiT():
            if 'p' not in memo:
                Bm = awphi_ref[pl.ds(4 * g, 4)].reshape(128, 32)
                Phi = jnp.where(blockmask, _mm(Bm, R), 0.0)
                memo['p'] = Phi.T.astype(bf16)
            return memo['p']

        def fold(part, k):
            def f(inj=False):
                r = _mm(phiT(), wraw[g, part, k * 128:(k + 1) * 128, :], NT)
                def fin():
                    WW[0, g, k, part * 128 // PW:(part + 1) * 128 // PW, :] = _pw(r.astype(bf16))
                if inj:
                    return None, fin
                fin()
            return f

        def vt(k):
            def f(inj=False):
                tt = _pw(wraw[g, 2, k * 128:(k + 1) * 128, :].T)
                def fin():
                    WW[0, g, k, 256 // PW:384 // PW, :] = tt
                if inj:
                    return tt, fin
                fin()
            return f
        out = []
        for k in range(8):
            out += ([fold(0, k), fold(1, k)] if 'f' in PP else []) + ([vt(k)] if 't' in PP else [])
        return out

    def prep_rest_pieces(g):
        def wo(t, k):
            def f(inj=False):
                tt = _pw(oraw[t, g, :, k * 128:(k + 1) * 128].T)
                def fin():
                    WO[t, g, k * 128 // PW:(k + 1) * 128 // PW, :] = tt
                if inj:
                    return tt, fin
                fin()
            return f

        def wb(part, k):
            def f(inj=False):
                tt = _pw(wraw[g, 4 + part, k * 128:(k + 1) * 128, :].T)
                def fin():
                    WW[1, g, k, part * 128 // PW:(part + 1) * 128 // PW, :] = tt
                if inj:
                    return tt, fin
                fin()
            return f
        out = []
        for k in range(8):
            out += [wo(0, k), wb(0, k), wb(1, k), wb(2, k), wo(1, k)] if 't' in PP else []
        return out

    def start(cs):
        for c in cs:
            c.start()

    def wait(cs):
        for c in cs:
            c.wait()

    if full:
        start([x_copy(c) for c in range(8)])
        start(wa_copies(0))
        for c in range(8):
            x_copy(c).wait()
            stage[c] = pltpu.bitcast(xraw[c], u32)
            for i in range(8):
                wd = stage.at[c][pl.ds(i, 128, stride=8), :].T
                xT[2 * i, c * 128:(c + 1) * 128, :] = pltpu.bitcast(wd << 16, f32)
                xT[2 * i + 1, c * 128:(c + 1) * 128, :] = pltpu.bitcast(wd & jnp.uint32(0xFFFF0000), f32)
            if c == 3:
                start(wa_copies(1) + rest_copies(0))
        wait(wa_copies(0))
        for f in prep_wa_pieces(0):
            f()

    lane = jax.lax.broadcasted_iota(jnp.int32, (4, 1, 128), 2)
    lane0 = lane == 0
    ones16 = jnp.ones((16, 128), f32)
    zero_u = zref[...]

    def ln_step(j):
        x = xT[j]
        m = jnp.sum(x, axis=0, keepdims=True) * (1.0 / D)
        xc = x - m
        v = jnp.sum(xc * xc, axis=0, keepdims=True) * (1.0 / D)
        lnT[j] = (xc * jax.lax.rsqrt(v + 1e-5)).astype(bf16)

    TN = (((0,), (0,)), ((), ()))

    def proj(lt, g, j):
        if lt == 1 and 'tnp' in CFG:
            return _mm(jnp.concatenate([wraw[g, 4 + p] for p in range(3)], axis=1), lnT[j], TN)
        return _mm(jnp.concatenate([_uw(WW[lt, g, k]) for k in range(8)], axis=1), lnT[j])

    def out_proj(lt, g, j, o):
        n = 1024 // OSPLIT
        for q in range(OSPLIT):
            if 'tno' in CFG:
                xT[j, q * n:(q + 1) * n, :] += _mm(oraw[lt, g, :, q * n:(q + 1) * n], o, TN)
                continue
            xT[j, q * n:(q + 1) * n, :] += _mm(_uw(WO[lt, g, q * n // PW:(q + 1) * n // PW, :]), o)

    def kv_step(pk, v, acc):
        t0, t1 = _phi(pk)
        l0 = jnp.concatenate([v[0:64], ones16], axis=0).astype(bf16)
        l1 = jnp.concatenate([v[64:128], ones16], axis=0).astype(bf16)
        a0 = _mm(l0, t0, NT)
        a1 = _mm(l1, t1, NT)
        if acc is None:
            return a0, a1
        return acc[0] + a0, acc[1] + a1

    rr = jax.lax.broadcasted_iota(jnp.int32, (80, 128), 0)
    cc = jax.lax.broadcasted_iota(jnp.int32, (80, 128), 1)
    row_head = jnp.where(rr < 64, rr // 32, (rr - 64) // 8)
    kvmask = row_head == ((cc // 32) % 2)

    def kv_final(acc, slot):
        lhsA[slot, 0] = _pk(jnp.where(kvmask, acc[0], 0.0).astype(bf16))
        lhsA[slot, 1] = _pk(jnp.where(kvmask, acc[1], 0.0).astype(bf16))

    def num_step(pq, slot, deps=()):
        t0, t1 = _phi(pq)
        outs = []
        for p, t in ((0, t0), (1, t1)):
            lw = lhsA[slot, p]
            if p == 0:
                z = None
                for dv in deps:
                    if dv is not None:
                        z = dv[56:64, :] if z is None else z | dv[56:64, :]
                if z is not None:
                    lw = jnp.concatenate([lw[0:8] | (z & zero_u), lw[8:]], axis=0)
            r = _mm(_up(lw), t)
            for hh in range(2):
                den = r[64 + 8 * hh: 72 + 8 * hh] + 1e-6
                num = r[32 * hh: 32 * hh + 32].reshape(4, 8, 128)
                outs.append((num * _recip(den)[None]).reshape(32, 128))
        return jnp.concatenate(outs, axis=0).astype(bf16)

    def att_tile(slot, j, kcache, vcache):
        def get(cache, base, jj):
            if jj not in cache:
                if jj >= 0:
                    cache[jj] = pbuf[slot, jj, base:base + 128, :]
                else:
                    cache[jj] = pltpu.roll(pbuf[slot, jj + 16, base:base + 128, :], 1, 1)
            return cache[jj]
        def one(h0, nh, dep):
            rows = lambda base: slice(base + 32 * h0, base + 32 * (h0 + nh))
            q = pbuf[slot, j, rows(0), :].reshape(nh, 32, 128)
            if dep is not None:
                q = q + dep
            ls = []
            for w in range(W):
                jj = j - DIL * w
                kk = get(kcache, 128, jj)[32 * h0: 32 * (h0 + nh)].reshape(nh, 32, 128)
                if 'wchain' in CFG and w > 0 and w % WC == 0:
                    qq = q + ls[-1][0:1] * 0.0
                else:
                    qq = q
                l = jnp.sum(qq * kk, axis=1, keepdims=True) * SCALE
                if jj < 0:
                    l = jnp.where(lane0[:nh], -1e9, l)
                ls.append(l)
            m = ls[0]
            for w in range(1, W):
                m = jnp.maximum(m, ls[w])
            es = [jnp.exp(l - m) for l in ls]
            ssum = es[0]
            for w in range(1, W):
                ssum = ssum + es[w]
            r = _recip(ssum)
            o = None
            for w in range(W):
                vv = get(vcache, 256, j - DIL * w)[32 * h0: 32 * (h0 + nh)].reshape(nh, 32, 128)
                t = (es[w] * r) * vv
                o = t if o is None else o + t
            return o
        if 'chain' in CFG:
            nh = 2 if 'chain2' in CFG else 1
            outs = []
            dep = None
            for h0 in range(0, 4, nh):
                o = one(h0, nh, dep)
                dep = o[0:1, 0:1, :] * 0.0
                outs.append(o.reshape(32 * nh, 128))
            return jnp.concatenate(outs, axis=0).astype(bf16)
        return one(0, 4, None).reshape(128, 128).astype(bf16)

    def block(front, back, ln, prep=()):
        st = {'acc': None}
        pend, ots = {}, {}
        kc, vc = {}, {}
        ft = front[0] if front else None
        bt = back[0] if back else None
        order = list(range(NJ - 1, -1, -1)) if bt == 'B' else list(range(NJ))

        def P(j):
            _, g, slot = front
            if ln:
                ln_step(j)
            r = proj(0 if ft == 'A' else 1, g, j)
            if ft == 'A':
                pbuf[slot, j, 0:128, :] = r[0:128]
                pend[j] = (r[128:256], r[256:384])
            else:
                pbuf[slot, j] = r

        def KV(j):
            pk, v = pend.pop(j)
            st['acc'] = kv_step(pk, v, st['acc'])

        def NUM(j):
            _, g, slot = back
            ots[j] = num_step(pbuf[slot, j, 0:128, :], slot, list(deps))
            del deps[:]

        def O(j):
            _, g, slot = back
            if bt == 'A':
                out_proj(0, g, j, ots.pop(j))
            else:
                out_proj(1, g, j, att_tile(slot, j, kc, vc))

        psk = PSK if (ln and back) else 0
        prep = list(prep)
        later, deps = [], []
        per = -(-len(prep) // NJ)
        for t in range(-1, NJ + psk + 2):
            def doprep(pos):
                if t >= 0 and pos == PREPPOS:
                    for f in prep[t * per:(t + 1) * per]:
                        if INJ:
                            v, fin = f(True)
                            later.append(fin)
                            deps.append(v)
                        else:
                            f()
            doprep(0)
            if bt == 'A' and 0 <= t + 1 < NJ:
                NUM(order[t + 1])
            doprep(1)
            if psk and 0 <= t < NJ:
                O(order[t])
            if front and 0 <= t - psk < NJ:
                P((order if ln or PORD else list(range(NJ)))[t - psk])
            doprep(2)
            if not psk and back and 0 <= t < NJ:
                O(order[t])
            doprep(3)
            if ft == 'A' and 0 <= t - psk - 1 < NJ:
                KV(order[t - psk - 1])
            doprep(4)
        if ft == 'A':
            kv_final(st['acc'], front[2])
        for fin in later:
            fin()
        if PREPPOS == 9:
            for f in prep:
                f()

    def a_loop(first):
        def body(g, _):
            slot = g % 2
            prep = ()
            if first:
                gn = jnp.minimum(g + 1, NG - 1)
                gnn = jnp.minimum(g + 2, NG - 1)
                @pl.when(g + 1 < NG)
                def _():
                    wait(wa_copies(g + 1))
                    start(rest_copies(g + 1))
                @pl.when(g + 2 < NG)
                def _():
                    start(wa_copies(g + 2))
                wait(rest_copies(g))
                prep = prep_wa_pieces(gn) + prep_rest_pieces(g)
            block(('A', g, slot), ('A', g - 1, 1 - slot), False, prep)
            return 0
        jax.lax.fori_loop(1, NG, body, 0)

    def b_loop():
        def body(g, _):
            slot = g % 2
            block(('B', g, slot), ('B', g - 1, 1 - slot), False)
            return 0
        jax.lax.fori_loop(1, NG, body, 0)

    L = (NG - 1) % 2
    if PART == 'A':
        a_loop(False)
    elif PART == 'A1':
        a_loop(True)
    elif PART == 'B':
        b_loop()
    elif PART == 'BS':
        block(('B', 1, 0), ('B', 0, 1), False)
    elif PART == 'AS':
        block(('A', 1, 0), ('A', 0, 1), False)
    elif PART == 'AB':
        block(('B', 0, 0), ('A', NG - 1, L), True)
    elif PART == 'BA':
        block(('A', 0, 0), ('B', NG - 1, L), True)
    elif PART == 'INIT':
        block(('A', 0, 0), None, True)
    elif PART == 'FIN':
        block(None, ('B', NG - 1, L), False)
    else:
        wait(wa_copies(1))
        start(wa_copies(2))
        wait(rest_copies(0))
        start(rest_copies(1))
        block(('A', 0, 0), None, True, prep_wa_pieces(1) + prep_rest_pieces(0))
        a_loop(True)
        block(('B', 0, 0), ('A', NG - 1, L), True)
        b_loop()
        block(('A', 0, 0), ('B', NG - 1, L), True)
        a_loop(False)
        block(('B', 0, 0), ('A', NG - 1, L), True)
        b_loop()
        block(None, ('B', NG - 1, L), False)

    if PART != 'ALL':
        acc = jnp.zeros((128, 128), f32)
        for j in range(NJ):
            acc = acc + xT[j, 0:128, :] + xT[j, 896:1024, :] + pbuf[0, j, 0:128, :] + pltpu.bitcast(lhsA[0, 0, 0:8, :], f32)[0:1]
        xraw[0, 0:128, :] = acc.astype(bf16)
        pltpu.sync_copy(xraw.at[0], out_hbm.at[:, 0:128])
        return
    def o_copy(c):
        return pltpu.make_async_copy(xraw.at[c], out_hbm.at[:, pl.ds(c * 128, 128)], sems.at[0, c])

    for c in range(8):
        for i in range(8):
            lo = xT[2 * i, c * 128:(c + 1) * 128, :]
            hi = xT[2 * i + 1, c * 128:(c + 1) * 128, :]
            lo = pltpu.bitcast(lo.astype(bf16).astype(f32), u32) >> 16
            hi = pltpu.bitcast(hi.astype(bf16).astype(f32), u32)
            stage.at[c][pl.ds(i, 128, stride=8), :] = (lo | hi).T
        xraw[c] = pltpu.bitcast(stage[c], bf16)
        o_copy(c).start()
    for c in range(8):
        o_copy(c).wait()


@jax.jit
def pallas_interleave_layers__linear_kernel_hedgehog__sliding_local_dilated__prompt_kernel(
    A_x, A_wqkv, A_w_phi, A_wo, B_x, B_wqkv, B_wo):
    del B_x
    x2 = A_x.reshape(S, D)
    hbm = pl.BlockSpec(memory_space=pl.ANY)
    out = pl.pallas_call(
        _kernel,
        out_shape=jax.ShapeDtypeStruct((S, D), bf16),
        in_specs=[hbm, hbm, pl.BlockSpec(memory_space=pltpu.VMEM), hbm, hbm, hbm],
        out_specs=hbm,
        scratch_shapes=[
            pltpu.VMEM((NJ, D, 128), f32),
            pltpu.VMEM((NJ, D, 128), bf16),
            pltpu.VMEM((2, NG, 8, 384 // PW, 128), bf16 if WBF else u32),
            pltpu.VMEM((2, NG, D // PW, 128), bf16 if WBF else u32),
            pltpu.VMEM((2, NJ, 384, 128), f32),
            pltpu.VMEM((2, 2, 40, 128), u32),
            pltpu.VMEM((8, S // 2, 128), u32),
            pltpu.VMEM((8, S, 128), bf16),
            pltpu.VMEM((NG, 7, D, 128), bf16),
            pltpu.VMEM((2, NG, 128, D), bf16),
            pltpu.VMEM((8, 128), u32),
            pltpu.SemaphoreType.DMA((9, 8)),
        ],
        compiler_params=pltpu.CompilerParams(vmem_limit_bytes=100 * 1024 * 1024, flags=FLAGS),
    )(x2, A_wqkv, A_w_phi, A_wo, B_wqkv, B_wo)
    return out.reshape(1, S, D)
```

```python
import jax
import jax.numpy as jnp
import jax.experimental.pallas as pl
import jax.experimental.pallas.tpu as pltpu

f32 = jnp.float32
bf16 = jnp.bfloat16
u32 = jnp.uint32

S, D, H, DH = 2048, 1024, 32, 32
PART = 'ALL'
CFG = 'sm'
FLAGS = None
WC = int('4')
OSPLIT = int('4')
PSK = int('1')
PORD = int('0')
PREPPOS = int('9')
PP = 'ft'
INJ = int('0')
PRESH = int('0')
OFIRST = int('0')
XS = int('5')
NG = 8
NJ = 16
W, DIL = 8, 2
SCALE = float(DH) ** -0.5
NT = (((1,), (1,)), ((), ()))


NN = (((1,), (0,)), ((), ()))


def _mm(a, b, dims=NN):
    return jax.lax.dot_general(a, b, dims, preferred_element_type=f32)


WBF = '0' == '1'
PW = 1 if WBF else 2


def _pw(x):
    return x if WBF else pltpu.bitcast(x, u32)


def _uw(x):
    return x if WBF else pltpu.bitcast(x, bf16)


def _pk(x):
    return pltpu.bitcast(x, u32)


def _up(x):
    return pltpu.bitcast(x, bf16)


def _recip(x):
    r = pl.reciprocal(x, approx=True)
    return r * (2.0 - x * r)


def _phi(p):
    p3 = p.reshape(4, 32, 128)
    mx = jnp.max(p3, axis=1, keepdims=True)
    mn = jnp.min(p3, axis=1, keepdims=True)
    e1 = jnp.exp(p3 - mx)
    e2 = jnp.exp(mn - p3)
    s1 = jnp.sum(e1, axis=1, keepdims=True)
    s2 = jnp.sum(e2, axis=1, keepdims=True)
    a = (e1 * _recip(s1)).reshape(128, 128)
    b = (e2 * _recip(s2)).reshape(128, 128)
    t0 = jnp.concatenate([a[0:64], b[0:64]], axis=0).astype(bf16)
    t1 = jnp.concatenate([a[64:128], b[64:128]], axis=0).astype(bf16)
    return t0, t1


def _kernel(x_hbm, awqkv_hbm, awphi_ref, awo_hbm, bwqkv_hbm, bwo_hbm, out_hbm,
            xT, lnT, WW, WO, pbuf, lhsA, stage, xraw, wraw, oraw, zref, shbuf, sems):
    zref[...] = jnp.zeros((8, 128), u32)
    full = PART == 'ALL'

    def x_copy(c):
        return pltpu.make_async_copy(x_hbm.at[:, pl.ds(c * 128, 128)], xraw.at[c], sems.at[0, c])

    def col(hbm, part, g):
        return hbm.at[:, pl.ds(pl.multiple_of(part * D + g * 128, 128), 128)]

    def wa_copies(g):
        return [pltpu.make_async_copy(col(awqkv_hbm, p, g), wraw.at[g, p], sems.at[1 + p, g]) for p in range(3)]

    def wb_copies(g):
        return [pltpu.make_async_copy(col(bwqkv_hbm, p, g), wraw.at[g, 4 + p], sems.at[5 + p, g]) for p in range(3)]

    def wo_copies(g):
        rows = pl.ds(pl.multiple_of(g * 128, 128), 128)
        return [pltpu.make_async_copy(awo_hbm.at[rows, :], oraw.at[0, g], sems.at[4, g]),
                pltpu.make_async_copy(bwo_hbm.at[rows, :], oraw.at[1, g], sems.at[8, g])]

    def rest_copies(g):
        return wo_copies(g) + wb_copies(g)

    f_i = jax.lax.broadcasted_iota(jnp.int32, (32, 128), 0)
    c_i = jax.lax.broadcasted_iota(jnp.int32, (32, 128), 1)
    R = jnp.where(c_i % 32 == f_i, 1.0, 0.0).astype(bf16)
    r2 = jax.lax.broadcasted_iota(jnp.int32, (128, 128), 0)
    c2 = jax.lax.broadcasted_iota(jnp.int32, (128, 128), 1)
    blockmask = (r2 // 32) == (c2 // 32)

    def prep_wa_pieces(g):
        memo = {}

        def phiT():
            if 'p' not in memo:
                Bm = awphi_ref[pl.ds(4 * g, 4)].reshape(128, 32)
                Phi = jnp.where(blockmask, _mm(Bm, R), 0.0)
                memo['p'] = Phi.T.astype(bf16)
            return memo['p']

        def fold(part, k):
            def f(inj=False):
                r = _mm(phiT(), wraw[g, part, k * 128:(k + 1) * 128, :], NT)
                def fin():
                    WW[0, g, k, part * 128 // PW:(part + 1) * 128 // PW, :] = _pw(r.astype(bf16))
                if inj:
                    return None, fin
                fin()
            return f

        def vt(k):
            def f(inj=False):
                tt = _pw(wraw[g, 2, k * 128:(k + 1) * 128, :].T)
                def fin():
                    WW[0, g, k, 256 // PW:384 // PW, :] = tt
                if inj:
                    return tt, fin
                fin()
            return f
        out = []
        for k in range(8):
            out += ([fold(0, k), fold(1, k)] if 'f' in PP else []) + ([vt(k)] if 't' in PP else [])
        return out

    def prep_rest_pieces(g):
        def wo(t, k):
            def f(inj=False):
                tt = _pw(oraw[t, g, :, k * 128:(k + 1) * 128].T)
                def fin():
                    WO[t, g, k * 128 // PW:(k + 1) * 128 // PW, :] = tt
                if inj:
                    return tt, fin
                fin()
            return f

        def wb(part, k):
            def f(inj=False):
                tt = _pw(wraw[g, 4 + part, k * 128:(k + 1) * 128, :].T)
                def fin():
                    WW[1, g, k, part * 128 // PW:(part + 1) * 128 // PW, :] = tt
                if inj:
                    return tt, fin
                fin()
            return f
        out = []
        for k in range(8):
            out += [wo(0, k), wb(0, k), wb(1, k), wb(2, k), wo(1, k)] if 't' in PP else []
        return out

    def start(cs):
        for c in cs:
            c.start()

    def wait(cs):
        for c in cs:
            c.wait()

    if full:
      with jax.named_scope('s0_prologue'):
        start(wa_copies(0))
        start([x_copy(c) for c in range(8)])
        wait(wa_copies(0))
        for f in prep_wa_pieces(0):
            f()
        for c in range(8):
            x_copy(c).wait()
            stage[c] = pltpu.bitcast(xraw[c], u32)
            for i in range(8):
                wd = stage.at[c][pl.ds(i, 128, stride=8), :].T
                xT[2 * i, c * 128:(c + 1) * 128, :] = pltpu.bitcast(wd << 16, f32)
                xT[2 * i + 1, c * 128:(c + 1) * 128, :] = pltpu.bitcast(wd & jnp.uint32(0xFFFF0000), f32)
            if c == XS:
                start(wa_copies(1) + rest_copies(0))

    lane = jax.lax.broadcasted_iota(jnp.int32, (4, 1, 128), 2)
    lane0 = lane == 0
    ones16 = jnp.ones((16, 128), f32)
    odd8 = (jax.lax.broadcasted_iota(jnp.int32, (8, 128), 0) % 2) == 1
    lane0_8 = jax.lax.broadcasted_iota(jnp.int32, (8, 128), 1) == 0
    zero_u = zref[...]

    def ln_step(j):
        x = xT[j]
        m = jnp.sum(x, axis=0, keepdims=True) * (1.0 / D)
        xc = x - m
        v = jnp.sum(xc * xc, axis=0, keepdims=True) * (1.0 / D)
        lnT[j] = (xc * jax.lax.rsqrt(v + 1e-5)).astype(bf16)

    TN = (((0,), (0,)), ((), ()))

    def proj(lt, g, j):
        if lt == 1 and 'tnp' in CFG:
            return _mm(jnp.concatenate([wraw[g, 4 + p] for p in range(3)], axis=1), lnT[j], TN)
        return _mm(jnp.concatenate([_uw(WW[lt, g, k]) for k in range(8)], axis=1), lnT[j])

    def out_proj(lt, g, j, o):
        n = 1024 // OSPLIT
        for q in range(OSPLIT):
            if 'tno' in CFG:
                xT[j, q * n:(q + 1) * n, :] += _mm(oraw[lt, g, :, q * n:(q + 1) * n], o, TN)
                continue
            xT[j, q * n:(q + 1) * n, :] += _mm(_uw(WO[lt, g, q * n // PW:(q + 1) * n // PW, :]), o)

    def kv_step(pk, v, acc):
        t0, t1 = _phi(pk)
        l0 = jnp.concatenate([v[0:64], ones16], axis=0).astype(bf16)
        l1 = jnp.concatenate([v[64:128], ones16], axis=0).astype(bf16)
        a0 = _mm(l0, t0, NT)
        a1 = _mm(l1, t1, NT)
        if acc is None:
            return a0, a1
        return acc[0] + a0, acc[1] + a1

    rr = jax.lax.broadcasted_iota(jnp.int32, (80, 128), 0)
    cc = jax.lax.broadcasted_iota(jnp.int32, (80, 128), 1)
    row_head = jnp.where(rr < 64, rr // 32, (rr - 64) // 8)
    kvmask = row_head == ((cc // 32) % 2)

    def kv_final(acc, slot):
        lhsA[slot, 0] = _pk(jnp.where(kvmask, acc[0], 0.0).astype(bf16))
        lhsA[slot, 1] = _pk(jnp.where(kvmask, acc[1], 0.0).astype(bf16))

    def num_step(pq, slot, deps=()):
        t0, t1 = _phi(pq)
        outs = []
        for p, t in ((0, t0), (1, t1)):
            lw = lhsA[slot, p]
            if p == 0:
                z = None
                for dv in deps:
                    if dv is not None:
                        z = dv[56:64, :] if z is None else z | dv[56:64, :]
                if z is not None:
                    lw = jnp.concatenate([lw[0:8] | (z & zero_u), lw[8:]], axis=0)
            r = _mm(_up(lw), t)
            for hh in range(2):
                den = r[64 + 8 * hh: 72 + 8 * hh] + 1e-6
                num = r[32 * hh: 32 * hh + 32].reshape(4, 8, 128)
                outs.append((num * _recip(den)[None]).reshape(32, 128))
        return jnp.concatenate(outs, axis=0).astype(bf16)

    def att_tile(slot, j, kcache, vcache):
        def get(cache, base, jj):
            if jj not in cache:
                if jj >= 0:
                    cache[jj] = pbuf[slot, jj, base:base + 128, :]
                else:
                    if PRESH:
                        cache[jj] = shbuf[slot, jj + 16, base - 128:base, :]
                    else:
                        cache[jj] = pltpu.roll(pbuf[slot, jj + 16, base:base + 128, :], 1, 1)
            return cache[jj]
        def one(h0, nh, dep):
            rows = lambda base: slice(base + 32 * h0, base + 32 * (h0 + nh))
            q = pbuf[slot, j, rows(0), :].reshape(nh, 32, 128)
            if dep is not None:
                q = q + dep
            ls = []
            for w in range(W):
                jj = j - DIL * w
                kk = get(kcache, 128, jj)[32 * h0: 32 * (h0 + nh)].reshape(nh, 32, 128)
                if 'wchain' in CFG and w > 0 and w % WC == 0:
                    qq = q + ls[-1][0:1] * 0.0
                else:
                    qq = q
                l = jnp.sum(qq * kk, axis=1, keepdims=True) * SCALE
                if jj < 0:
                    l = jnp.where(lane0[:nh], -1e9, l)
                ls.append(l)
            m = ls[0]
            for w in range(1, W):
                m = jnp.maximum(m, ls[w])
            es = [jnp.exp(l - m) for l in ls]
            ssum = es[0]
            for w in range(1, W):
                ssum = ssum + es[w]
            r = _recip(ssum)
            o = None
            for w in range(W):
                vv = get(vcache, 256, j - DIL * w)[32 * h0: 32 * (h0 + nh)].reshape(nh, 32, 128)
                t = (es[w] * r) * vv
                o = t if o is None else o + t
            return o
        if 'sm' in CFG:
            q = pbuf[slot, j, 0:128, :].reshape(16, 8, 128)
            ls = []
            for w in range(W):
                jj = j - DIL * w
                kk = get(kcache, 128, jj).reshape(16, 8, 128)
                a = jnp.sum(q * kk, axis=0)
                l = (a + pltpu.roll(a, 4, 0)) * SCALE
                if jj < 0:
                    l = jnp.where(lane0_8, -1e9, l)
                ls.append(l)
            m = ls[0]
            for w in range(1, W):
                m = jnp.maximum(m, ls[w])
            es = [jnp.exp(l - m) for l in ls]
            ssum = es[0]
            for w in range(1, W):
                ssum = ssum + es[w]
            r = _recip(ssum)
            if 'smv' in CFG:
                o = None
                for w in range(W):
                    vv = get(vcache, 256, j - DIL * w).reshape(16, 8, 128)
                    t = (es[w] * r)[None] * vv
                    o = t if o is None else o + t
                return o.reshape(128, 128).astype(bf16)
            outs = []
            aw = [es[w] * r for w in range(W)]
            for hh in range(4):
                o = None
                for w in range(W):
                    vv = get(vcache, 256, j - DIL * w)[32 * hh:32 * hh + 32].reshape(4, 8, 128)
                    t = aw[w][hh:hh + 1][None] * vv
                    o = t if o is None else o + t
                outs.append(o.reshape(32, 128))
            return jnp.concatenate(outs, axis=0).astype(bf16)
        if 'dm' in CFG:
            q = pbuf[slot, j, 0:128, :].reshape(16, 8, 128)
            ls = []
            for w in range(W):
                jj = j - DIL * w
                kk = get(kcache, 128, jj).reshape(16, 8, 128)
                a = jnp.sum(q * kk, axis=0)
                l = (a + jnp.where(odd8, pltpu.roll(a, 1, 0), pltpu.roll(a, 7, 0))) * SCALE
                if jj < 0:
                    l = jnp.where(lane0_8, -1e9, l)
                ls.append(l)
            m = ls[0]
            for w in range(1, W):
                m = jnp.maximum(m, ls[w])
            es = [jnp.exp(l - m) for l in ls]
            ssum = es[0]
            for w in range(1, W):
                ssum = ssum + es[w]
            r = _recip(ssum)
            o = None
            for w in range(W):
                vv = get(vcache, 256, j - DIL * w).reshape(16, 8, 128)
                t = (es[w] * r)[None] * vv
                o = t if o is None else o + t
            return o.reshape(128, 128).astype(bf16)
        if 'chain' in CFG:
            nh = 2 if 'chain2' in CFG else 1
            outs = []
            dep = None
            for h0 in range(0, 4, nh):
                o = one(h0, nh, dep)
                dep = o[0:1, 0:1, :] * 0.0
                outs.append(o.reshape(32 * nh, 128))
            return jnp.concatenate(outs, axis=0).astype(bf16)
        return one(0, 4, None).reshape(128, 128).astype(bf16)

    def block(front, back, ln, prep=()):
        st = {'acc': None}
        pend, ots = {}, {}
        kc, vc = {}, {}
        ft = front[0] if front else None
        bt = back[0] if back else None
        order = list(range(NJ - 1, -1, -1)) if bt == 'B' else list(range(NJ))

        def P(j):
            _, g, slot = front
            if ln:
                ln_step(j)
            r = proj(0 if ft == 'A' else 1, g, j)
            if ft == 'A':
                pbuf[slot, j, 0:128, :] = r[0:128]
                pend[j] = (r[128:256], r[256:384])
            else:
                if 'sm' in CFG:
                    np_ = 3 if 'smv' in CFG else 2
                    for part in range(np_):
                        for hh in range(4):
                            for a in range(4):
                                r0 = part * 128 + hh * 32 + a * 8
                                pbuf.at[slot, j][pl.ds(part * 128 + 32 * a + hh, 8, stride=4), :] = r[r0:r0 + 8]
                    if np_ == 2:
                        pbuf[slot, j, 256:384, :] = r[256:384]
                else:
                    pbuf[slot, j, 0:384, :] = r
                if PRESH and j >= DIL:
                    shbuf[slot, j, 0:128, :] = pltpu.roll(r[128:256], 1, 1)
                    shbuf[slot, j, 128:256, :] = pltpu.roll(r[256:384], 1, 1)

        def KV(j):
            pk, v = pend.pop(j)
            st['acc'] = kv_step(pk, v, st['acc'])

        def NUM(j):
            _, g, slot = back
            ots[j] = num_step(pbuf[slot, j, 0:128, :], slot, list(deps))
            del deps[:]

        def O(j):
            _, g, slot = back
            if bt == 'A':
                out_proj(0, g, j, ots.pop(j))
            else:
                out_proj(1, g, j, att_tile(slot, j, kc, vc))

        psk = PSK if (ln and back) else 0
        prep = list(prep)
        later, deps = [], []
        per = -(-len(prep) // NJ)
        for t in range(-1, NJ + psk + 2):
            def doprep(pos):
                if t >= 0 and pos == PREPPOS:
                    for f in prep[t * per:(t + 1) * per]:
                        if INJ:
                            v, fin = f(True)
                            later.append(fin)
                            deps.append(v)
                        else:
                            f()
            doprep(0)
            if bt == 'A' and 0 <= t + 1 < NJ:
                NUM(order[t + 1])
            doprep(1)
            if (psk or OFIRST) and back and 0 <= t < NJ:
                O(order[t])
            if front and 0 <= t - psk < NJ:
                P((order if ln or PORD else list(range(NJ)))[t - psk])
            doprep(2)
            if not (psk or OFIRST) and back and 0 <= t < NJ:
                O(order[t])
            doprep(3)
            if ft == 'A' and 0 <= t - psk - 1 < NJ:
                KV(order[t - psk - 1])
            doprep(4)
        if ft == 'A':
            kv_final(st['acc'], front[2])
        for fin in later:
            fin()
        if PREPPOS == 9:
            for f in prep:
                f()

    def a_loop(first):
        def body(g, _):
            slot = g % 2
            prep = ()
            if first:
                gn = jnp.minimum(g + 1, NG - 1)
                gnn = jnp.minimum(g + 2, NG - 1)
                @pl.when(g + 1 < NG)
                def _():
                    wait(wa_copies(g + 1))
                    start(rest_copies(g + 1))
                @pl.when(g + 2 < NG)
                def _():
                    start(wa_copies(g + 2))
                wait(rest_copies(g))
                prep = prep_wa_pieces(gn) + prep_rest_pieces(g)
            block(('A', g, slot), ('A', g - 1, 1 - slot), False, prep)
            return 0
        jax.lax.fori_loop(1, NG, body, 0)

    def b_loop():
        def body(g, _):
            slot = g % 2
            block(('B', g, slot), ('B', g - 1, 1 - slot), False)
            return 0
        jax.lax.fori_loop(1, NG, body, 0)

    L = (NG - 1) % 2
    if PART == 'A':
        a_loop(False)
    elif PART == 'A1':
        a_loop(True)
    elif PART == 'B':
        b_loop()
    elif PART == 'BS':
        block(('B', 1, 0), ('B', 0, 1), False)
    elif PART == 'AS':
        block(('A', 1, 0), ('A', 0, 1), False)
    elif PART == 'AB':
        block(('B', 0, 0), ('A', NG - 1, L), True)
    elif PART == 'BA':
        block(('A', 0, 0), ('B', NG - 1, L), True)
    elif PART == 'INIT':
        block(('A', 0, 0), None, True)
    elif PART == 'FIN':
        block(None, ('B', NG - 1, L), False)
    else:
        with jax.named_scope("s1_init"):
            start(wa_copies(2) + rest_copies(1))

            def w0():
                wait(wa_copies(1))
                wait(rest_copies(0))
            block(('A', 0, 0), None, True, [w0] + prep_wa_pieces(1) + prep_rest_pieces(0))
        with jax.named_scope("s2_loopA1"):
            a_loop(True)
        with jax.named_scope("s3_AB"):
            block(('B', 0, 0), ('A', NG - 1, L), True)
        with jax.named_scope("s4_loopB"):
            b_loop()
        with jax.named_scope("s5_BA"):
            block(('A', 0, 0), ('B', NG - 1, L), True)
        with jax.named_scope("s6_loopA2"):
            a_loop(False)
        with jax.named_scope("s7_AB"):
            block(('B', 0, 0), ('A', NG - 1, L), True)
        with jax.named_scope("s8_loopB"):
            b_loop()
        with jax.named_scope("s9_fin"):
            block(None, ('B', NG - 1, L), False)

    if PART != 'ALL':
        acc = jnp.zeros((128, 128), f32)
        for j in range(NJ):
            acc = acc + xT[j, 0:128, :] + xT[j, 896:1024, :] + pbuf[0, j, 0:128, :] + pltpu.bitcast(lhsA[0, 0, 0:8, :], f32)[0:1]
        xraw[0, 0:128, :] = acc.astype(bf16)
        pltpu.sync_copy(xraw.at[0], out_hbm.at[:, 0:128])
        return
    def o_copy(c):
        return pltpu.make_async_copy(xraw.at[c], out_hbm.at[:, pl.ds(c * 128, 128)], sems.at[0, c])

    with jax.named_scope('sa_epilogue'):
      for c in range(8):
        for i in range(8):
            lo = xT[2 * i, c * 128:(c + 1) * 128, :]
            hi = xT[2 * i + 1, c * 128:(c + 1) * 128, :]
            lo = pltpu.bitcast(lo.astype(bf16).astype(f32), u32) >> 16
            hi = pltpu.bitcast(hi.astype(bf16).astype(f32), u32)
            stage.at[c][pl.ds(i, 128, stride=8), :] = (lo | hi).T
        xraw[c] = pltpu.bitcast(stage[c], bf16)
        o_copy(c).start()
      for c in range(8):
        o_copy(c).wait()


@jax.jit
def pallas_interleave_layers__linear_kernel_hedgehog__sliding_local_dilated__prompt_kernel(
    A_x, A_wqkv, A_w_phi, A_wo, B_x, B_wqkv, B_wo):
    del B_x
    x2 = A_x.reshape(S, D)
    hbm = pl.BlockSpec(memory_space=pl.ANY)
    out = pl.pallas_call(
        _kernel,
        out_shape=jax.ShapeDtypeStruct((S, D), bf16),
        in_specs=[hbm, hbm, pl.BlockSpec(memory_space=pltpu.VMEM), hbm, hbm, hbm],
        out_specs=hbm,
        scratch_shapes=[
            pltpu.VMEM((NJ, D, 128), f32),
            pltpu.VMEM((NJ, D, 128), bf16),
            pltpu.VMEM((2, NG, 8, 384 // PW, 128), bf16 if WBF else u32),
            pltpu.VMEM((2, NG, D // PW, 128), bf16 if WBF else u32),
            pltpu.VMEM((2, NJ, 384, 128), f32),
            pltpu.VMEM((2, 2, 40, 128), u32),
            pltpu.VMEM((8, S // 2, 128), u32),
            pltpu.VMEM((8, S, 128), bf16),
            pltpu.VMEM((NG, 7, D, 128), bf16),
            pltpu.VMEM((2, NG, 128, D), bf16),
            pltpu.VMEM((8, 128), u32),
            pltpu.VMEM((2, NJ, 256, 128), f32),
            pltpu.SemaphoreType.DMA((9, 8)),
        ],
        compiler_params=pltpu.CompilerParams(vmem_limit_bytes=100 * 1024 * 1024, flags=FLAGS),
    )(x2, A_wqkv, A_w_phi, A_wo, B_wqkv, B_wo)
    return out.reshape(1, S, D)
```

```python
import jax
import jax.numpy as jnp
import jax.experimental.pallas as pl
import jax.experimental.pallas.tpu as pltpu

f32 = jnp.float32
bf16 = jnp.bfloat16
u32 = jnp.uint32

S, D, H, DH = 2048, 1024, 32, 32
PART = 'ALL'
CFG = 'sm'
FLAGS = None
WC = int('4')
OSPLIT = int('4')
PSK = int('1')
PORD = int('0')
PREPPOS = int('9')
PP = 'ft'
INJ = int('0')
PRESH = int('0')
OFIRST = int('0')
XS = int('3')
XG = int('4')
NG = 8
NJ = 16
W, DIL = 8, 2
SCALE = float(DH) ** -0.5
NT = (((1,), (1,)), ((), ()))


NN = (((1,), (0,)), ((), ()))


def _mm(a, b, dims=NN):
    return jax.lax.dot_general(a, b, dims, preferred_element_type=f32)


PW = 1


def _pw(x):
    return x


def _uw(ref):
    return pltpu.bitcast(ref.bitcast(u32)[...], bf16)


def _pk(x):
    return pltpu.bitcast(x, u32)


def _up(x):
    return pltpu.bitcast(x, bf16)


def _recip(x):
    r = pl.reciprocal(x, approx=True)
    return r * (2.0 - x * r)


def _phi(p):
    p3 = p.reshape(4, 32, 128)
    mx = jnp.max(p3, axis=1, keepdims=True)
    mn = jnp.min(p3, axis=1, keepdims=True)
    e1 = jnp.exp(p3 - mx)
    e2 = jnp.exp(mn - p3)
    s1 = jnp.sum(e1, axis=1, keepdims=True)
    s2 = jnp.sum(e2, axis=1, keepdims=True)
    a = (e1 * _recip(s1)).reshape(128, 128)
    b = (e2 * _recip(s2)).reshape(128, 128)
    t0 = jnp.concatenate([a[0:64], b[0:64]], axis=0).astype(bf16)
    t1 = jnp.concatenate([a[64:128], b[64:128]], axis=0).astype(bf16)
    return t0, t1


def _kernel(x_hbm, awqkv_hbm, awphi_ref, awo_hbm, bwqkv_hbm, bwo_hbm, out_hbm,
            xT, lnT, WW, WO, pbuf, lhsA, xraw, wraw, oraw, zref, shbuf, sems):
    zref[...] = jnp.zeros((8, 128), u32)
    full = PART == 'ALL'

    def x_copy(c):
        return pltpu.make_async_copy(x_hbm.bitcast(u32).at[:, c, :], xraw.at[c], sems.at[0, c])

    def col(hbm, part, g):
        return hbm.at[:, pl.ds(pl.multiple_of(part * D + g * 128, 128), 128)]

    def wa_copies(g):
        return [pltpu.make_async_copy(col(awqkv_hbm, p, g), wraw.at[g, p], sems.at[1 + p, g]) for p in range(3)]

    def wb_copies(g):
        return [pltpu.make_async_copy(col(bwqkv_hbm, p, g), wraw.at[g, 4 + p], sems.at[5 + p, g]) for p in range(3)]

    def wo_copies(g):
        rows = pl.ds(pl.multiple_of(g * 128, 128), 128)
        return [pltpu.make_async_copy(awo_hbm.at[rows, :], oraw.at[0, g], sems.at[4, g]),
                pltpu.make_async_copy(bwo_hbm.at[rows, :], oraw.at[1, g], sems.at[8, g])]

    def rest_copies(g):
        return wo_copies(g) + wb_copies(g)

    f_i = jax.lax.broadcasted_iota(jnp.int32, (32, 128), 0)
    c_i = jax.lax.broadcasted_iota(jnp.int32, (32, 128), 1)
    R = jnp.where(c_i % 32 == f_i, 1.0, 0.0).astype(bf16)
    r2 = jax.lax.broadcasted_iota(jnp.int32, (128, 128), 0)
    c2 = jax.lax.broadcasted_iota(jnp.int32, (128, 128), 1)
    blockmask = (r2 // 32) == (c2 // 32)

    def build_w(lt, g):
        tiles = []
        if lt == 0:
            Bm = awphi_ref[pl.ds(4 * g, 4)].reshape(128, 32)
            Phi = jnp.where(blockmask, _mm(Bm, R), 0.0)
            PhiT = Phi.T.astype(bf16)
        for k in range(8):
            ks = slice(k * 128, (k + 1) * 128)
            if lt == 0:
                parts = [_mm(PhiT, wraw[g, 0, ks, :], NT).astype(bf16),
                         _mm(PhiT, wraw[g, 1, ks, :], NT).astype(bf16),
                         wraw[g, 2, ks, :].T]
            else:
                parts = [wraw[g, 4 + p, ks, :].T for p in range(3)]
            t = jnp.concatenate(parts, axis=0)
            WW[lt, g, k] = t
            tiles.append(t)
        return tiles

    def build_wo(lt, g, q, n):
        t = jnp.concatenate([oraw[lt, g, :, c * 128:(c + 1) * 128].T for c in range(q * n // 128, (q + 1) * n // 128)], axis=0)
        WO[lt, g, pl.ds(q * n, n), :] = t
        return t

    def start(cs):
        for c in cs:
            c.start()

    def wait(cs):
        for c in cs:
            c.wait()

    if full:
      with jax.named_scope('s0_prologue'):
        start(wa_copies(0))
        start([x_copy(c) for c in range(8)])
        wait(wa_copies(0))
        build_w(0, 0)

    def x_in(i):
        x_copy(i).wait()
        for c in range(8):
            wd = xraw[i, :, c * 128:(c + 1) * 128].T
            xT[2 * i, c * 128:(c + 1) * 128, :] = pltpu.bitcast(wd << 16, f32)
            xT[2 * i + 1, c * 128:(c + 1) * 128, :] = pltpu.bitcast(wd & jnp.uint32(0xFFFF0000), f32)

    def o_copy(i):
        return pltpu.make_async_copy(xraw.at[i], out_hbm.bitcast(u32).at[:, i, :], sems.at[0, i])

    def x_out(i):
        for c in range(8):
            lo = xT[2 * i, c * 128:(c + 1) * 128, :]
            hi = xT[2 * i + 1, c * 128:(c + 1) * 128, :]
            lo = pltpu.bitcast(lo.astype(bf16).astype(f32), u32) >> 16
            hi = pltpu.bitcast(hi.astype(bf16).astype(f32), u32)
            xraw[i, :, c * 128:(c + 1) * 128] = (lo | hi).T
        o_copy(i).start()

    lane = jax.lax.broadcasted_iota(jnp.int32, (4, 1, 128), 2)
    lane0 = lane == 0
    ones16 = jnp.ones((16, 128), f32)
    odd8 = (jax.lax.broadcasted_iota(jnp.int32, (8, 128), 0) % 2) == 1
    lane0_8 = jax.lax.broadcasted_iota(jnp.int32, (8, 128), 1) == 0
    zero_u = zref[...]

    def ln_step(j):
        x = xT[j]
        m = jnp.sum(x, axis=0, keepdims=True) * (1.0 / D)
        xc = x - m
        v = jnp.sum(xc * xc, axis=0, keepdims=True) * (1.0 / D)
        lnT[j] = (xc * jax.lax.rsqrt(v + 1e-5)).astype(bf16)

    TN = (((0,), (0,)), ((), ()))

    def proj(lt, g, j, build=False):
        if build:
            return _mm(jnp.concatenate(build_w(lt, g), axis=1), _uw(lnT.at[j]))
        if lt == 1 and 'tnp' in CFG:
            return _mm(jnp.concatenate([wraw[g, 4 + p] for p in range(3)], axis=1), lnT[j], TN)
        return _mm(jnp.concatenate([_uw(WW.at[lt, g, k]) for k in range(8)], axis=1), _uw(lnT.at[j]))

    def out_proj(lt, g, j, o, build=False):
        n = 1024 // OSPLIT
        for q in range(OSPLIT):
            if build:
                xT[j, q * n:(q + 1) * n, :] += _mm(build_wo(lt, g, q, n), o)
                continue
            if 'tno' in CFG:
                xT[j, q * n:(q + 1) * n, :] += _mm(oraw[lt, g, :, q * n:(q + 1) * n], o, TN)
                continue
            xT[j, q * n:(q + 1) * n, :] += _mm(_uw(WO.at[lt, g, pl.ds(q * n, n)]), o)

    def kv_step(pk, v, acc):
        t0, t1 = _phi(pk)
        l0 = jnp.concatenate([v[0:64], ones16], axis=0).astype(bf16)
        l1 = jnp.concatenate([v[64:128], ones16], axis=0).astype(bf16)
        a0 = _mm(l0, t0, NT)
        a1 = _mm(l1, t1, NT)
        if acc is None:
            return a0, a1
        return acc[0] + a0, acc[1] + a1

    rr = jax.lax.broadcasted_iota(jnp.int32, (80, 128), 0)
    cc = jax.lax.broadcasted_iota(jnp.int32, (80, 128), 1)
    row_head = jnp.where(rr < 64, rr // 32, (rr - 64) // 8)
    kvmask = row_head == ((cc // 32) % 2)

    def kv_final(acc, slot):
        lhsA[slot, 0] = _pk(jnp.where(kvmask, acc[0], 0.0).astype(bf16))
        lhsA[slot, 1] = _pk(jnp.where(kvmask, acc[1], 0.0).astype(bf16))

    def num_step(pq, slot, deps=()):
        t0, t1 = _phi(pq)
        outs = []
        for p, t in ((0, t0), (1, t1)):
            lw = lhsA[slot, p]
            if p == 0:
                z = None
                for dv in deps:
                    if dv is not None:
                        z = dv[56:64, :] if z is None else z | dv[56:64, :]
                if z is not None:
                    lw = jnp.concatenate([lw[0:8] | (z & zero_u), lw[8:]], axis=0)
            r = _mm(_up(lw), t)
            for hh in range(2):
                den = r[64 + 8 * hh: 72 + 8 * hh] + 1e-6
                num = r[32 * hh: 32 * hh + 32].reshape(4, 8, 128)
                outs.append((num * _recip(den)[None]).reshape(32, 128))
        return jnp.concatenate(outs, axis=0).astype(bf16)

    def att_tile(slot, j, kcache, vcache):
        def get(cache, base, jj):
            if jj not in cache:
                if jj >= 0:
                    cache[jj] = pbuf[slot, jj, base:base + 128, :]
                else:
                    if PRESH:
                        cache[jj] = shbuf[slot, jj + 16, base - 128:base, :]
                    else:
                        cache[jj] = pltpu.roll(pbuf[slot, jj + 16, base:base + 128, :], 1, 1)
            return cache[jj]
        def one(h0, nh, dep):
            rows = lambda base: slice(base + 32 * h0, base + 32 * (h0 + nh))
            q = pbuf[slot, j, rows(0), :].reshape(nh, 32, 128)
            if dep is not None:
                q = q + dep
            ls = []
            for w in range(W):
                jj = j - DIL * w
                kk = get(kcache, 128, jj)[32 * h0: 32 * (h0 + nh)].reshape(nh, 32, 128)
                if 'wchain' in CFG and w > 0 and w % WC == 0:
                    qq = q + ls[-1][0:1] * 0.0
                else:
                    qq = q
                l = jnp.sum(qq * kk, axis=1, keepdims=True) * SCALE
                if jj < 0:
                    l = jnp.where(lane0[:nh], -1e9, l)
                ls.append(l)
            m = ls[0]
            for w in range(1, W):
                m = jnp.maximum(m, ls[w])
            es = [jnp.exp(l - m) for l in ls]
            ssum = es[0]
            for w in range(1, W):
                ssum = ssum + es[w]
            r = _recip(ssum)
            o = None
            for w in range(W):
                vv = get(vcache, 256, j - DIL * w)[32 * h0: 32 * (h0 + nh)].reshape(nh, 32, 128)
                t = (es[w] * r) * vv
                o = t if o is None else o + t
            return o
        if 'sm' in CFG:
            q = pbuf[slot, j, 0:128, :].reshape(16, 8, 128)
            ls = []
            for w in range(W):
                jj = j - DIL * w
                kk = get(kcache, 128, jj).reshape(16, 8, 128)
                a = jnp.sum(q * kk, axis=0)
                l = (a + pltpu.roll(a, 4, 0)) * SCALE
                if jj < 0:
                    l = jnp.where(lane0_8, -1e9, l)
                ls.append(l)
            m = ls[0]
            for w in range(1, W):
                m = jnp.maximum(m, ls[w])
            es = [jnp.exp(l - m) for l in ls]
            ssum = es[0]
            for w in range(1, W):
                ssum = ssum + es[w]
            r = _recip(ssum)
            if 'smv' in CFG:
                o = None
                for w in range(W):
                    vv = get(vcache, 256, j - DIL * w).reshape(16, 8, 128)
                    t = (es[w] * r)[None] * vv
                    o = t if o is None else o + t
                return o.reshape(128, 128).astype(bf16)
            outs = []
            aw = [es[w] * r for w in range(W)]
            for hh in range(4):
                o = None
                for w in range(W):
                    vv = get(vcache, 256, j - DIL * w)[32 * hh:32 * hh + 32].reshape(4, 8, 128)
                    t = aw[w][hh:hh + 1][None] * vv
                    o = t if o is None else o + t
                outs.append(o.reshape(32, 128))
            return jnp.concatenate(outs, axis=0).astype(bf16)
        if 'dm' in CFG:
            q = pbuf[slot, j, 0:128, :].reshape(16, 8, 128)
            ls = []
            for w in range(W):
                jj = j - DIL * w
                kk = get(kcache, 128, jj).reshape(16, 8, 128)
                a = jnp.sum(q * kk, axis=0)
                l = (a + jnp.where(odd8, pltpu.roll(a, 1, 0), pltpu.roll(a, 7, 0))) * SCALE
                if jj < 0:
                    l = jnp.where(lane0_8, -1e9, l)
                ls.append(l)
            m = ls[0]
            for w in range(1, W):
                m = jnp.maximum(m, ls[w])
            es = [jnp.exp(l - m) for l in ls]
            ssum = es[0]
            for w in range(1, W):
                ssum = ssum + es[w]
            r = _recip(ssum)
            o = None
            for w in range(W):
                vv = get(vcache, 256, j - DIL * w).reshape(16, 8, 128)
                t = (es[w] * r)[None] * vv
                o = t if o is None else o + t
            return o.reshape(128, 128).astype(bf16)
        if 'chain' in CFG:
            nh = 2 if 'chain2' in CFG else 1
            outs = []
            dep = None
            for h0 in range(0, 4, nh):
                o = one(h0, nh, dep)
                dep = o[0:1, 0:1, :] * 0.0
                outs.append(o.reshape(32 * nh, 128))
            return jnp.concatenate(outs, axis=0).astype(bf16)
        return one(0, 4, None).reshape(128, 128).astype(bf16)

    def block(front, back, ln, prep=None, bw=False, bo=False, js=None, st0=None, fin=True):
        st = st0 if st0 is not None else {'acc': None, 'p1': False, 'o1': False}
        pend, ots = {}, {}
        kc, vc = st.setdefault('kc', {}), st.setdefault('vc', {})
        ft = front[0] if front else None
        bt = back[0] if back else None
        order = list(range(NJ - 1, -1, -1)) if bt == 'B' else list(range(NJ))

        def P(j):
            _, g, slot = front
            if ln:
                ln_step(j)
            r = proj(0 if ft == 'A' else 1, g, j, bw and not st['p1'])
            st['p1'] = True
            if ft == 'A':
                pbuf[slot, j, 0:128, :] = r[0:128]
                pend[j] = (r[128:256], r[256:384])
            else:
                if 'sm' in CFG:
                    np_ = 3 if 'smv' in CFG else 2
                    for part in range(np_):
                        for hh in range(4):
                            for a in range(4):
                                r0 = part * 128 + hh * 32 + a * 8
                                pbuf.at[slot, j][pl.ds(part * 128 + 32 * a + hh, 8, stride=4), :] = r[r0:r0 + 8]
                    if np_ == 2:
                        pbuf[slot, j, 256:384, :] = r[256:384]
                else:
                    pbuf[slot, j, 0:384, :] = r
                if PRESH and j >= DIL:
                    shbuf[slot, j, 0:128, :] = pltpu.roll(r[128:256], 1, 1)
                    shbuf[slot, j, 128:256, :] = pltpu.roll(r[256:384], 1, 1)

        def KV(j):
            pk, v = pend.pop(j)
            st['acc'] = kv_step(pk, v, st['acc'])

        def NUM(j):
            _, g, slot = back
            ots[j] = num_step(pbuf[slot, j, 0:128, :], slot)

        def O(j):
            _, g, slot = back
            if bt == 'A':
                out_proj(0, g, j, ots.pop(j), bo and not st['o1'])
                st['o1'] = True
            else:
                out_proj(1, g, j, att_tile(slot, j, kc, vc), bo and not st['o1'])
            st['o1'] = True

        if js is not None:
            order = list(js)
        n = len(order)
        psk = PSK if (ln and back) else 0
        for t in range(-1, n + psk + 2):
            if bt == 'A' and 0 <= t + 1 < n:
                NUM(order[t + 1])
            if (psk or OFIRST) and back and 0 <= t < n:
                O(order[t])
            if front and 0 <= t - psk < n:
                P((order if ln or PORD or js is not None else list(range(NJ)))[t - psk])
            if not (psk or OFIRST) and back and 0 <= t < n:
                O(order[t])
            if ft == 'A' and 0 <= t - psk - 1 < n:
                KV(order[t - psk - 1])
        if ft == 'A' and fin:
            kv_final(st['acc'], front[2])
        if prep is not None:
            prep()

    def prep_next(g, gn):
        build_w(0, gn)
        build_wo(0, g, 0, 1024)
        build_w(1, g)
        build_wo(1, g, 0, 1024)

    def a_loop(first):
        def body(g, _):
            slot = g % 2
            prep = None
            if first:
                @pl.when(g + 1 < NG)
                def _():
                    wait(wa_copies(g + 1))
                    start(rest_copies(g + 1))

                @pl.when(g + 2 < NG)
                def _():
                    start(wa_copies(g + 2))
                wait(rest_copies(g))
                prep = lambda: prep_next(g, jnp.minimum(g + 1, NG - 1))
            block(('A', g, slot), ('A', g - 1, 1 - slot), False, prep)
            return 0
        jax.lax.fori_loop(1, NG, body, 0)

    def b_loop(first):
        def body(g, _):
            slot = g % 2
            block(('B', g, slot), ('B', g - 1, 1 - slot), False)
            return 0
        jax.lax.fori_loop(1, NG, body, 0)

    L = (NG - 1) % 2
    if PART == 'A':
        a_loop(False)
    elif PART == 'A1':
        a_loop(True)
    elif PART == 'B':
        b_loop(False)
    elif PART == 'B1':
        b_loop(True)
    elif PART == 'BS':
        block(('B', 1, 0), ('B', 0, 1), False)
    elif PART == 'AS':
        block(('A', 1, 0), ('A', 0, 1), False)
    elif PART == 'AB':
        block(('B', 0, 0), ('A', NG - 1, L), True)
    elif PART == 'BA':
        block(('A', 0, 0), ('B', NG - 1, L), True)
    elif PART == 'INIT':
        block(('A', 0, 0), None, True)
    elif PART == 'FIN':
        block(None, ('B', NG - 1, L), False)
    else:
        sti = {'acc': None, 'p1': False, 'o1': False}
        for h in range(8 // XG):
            with jax.named_scope("s1_init"):
                for i in range(h * XG, (h + 1) * XG):
                    x_in(i)
                    if i == XS:
                        start(wa_copies(1) + rest_copies(0))
            with jax.named_scope("s1_initb"):
                last = h == 8 // XG - 1
                if last:
                    start(wa_copies(2) + rest_copies(1))

                def prep0():
                    wait(wa_copies(1) + rest_copies(0))
                    prep_next(0, 1)
                block(('A', 0, 0), None, True, prep0 if last else None, js=range(2 * XG * h, 2 * XG * (h + 1)), st0=sti, fin=last)
        with jax.named_scope("s2_loopA1"):
            a_loop(True)
        with jax.named_scope("s3_AB"):
            block(('B', 0, 0), ('A', NG - 1, L), True)
        with jax.named_scope("s4_loopB1"):
            b_loop(True)
        with jax.named_scope("s5_BA"):
            block(('A', 0, 0), ('B', NG - 1, L), True)
        with jax.named_scope("s6_loopA2"):
            a_loop(False)
        with jax.named_scope("s7_AB"):
            block(('B', 0, 0), ('A', NG - 1, L), True)
        with jax.named_scope("s8_loopB"):
            b_loop(False)
        stf = {'acc': None, 'p1': False, 'o1': False}
        for i in range(7, -1, -1):
            with jax.named_scope("s9_fin"):
                block(None, ('B', NG - 1, L), False, js=(2 * i + 1, 2 * i), st0=stf)
                if i < 7:
                    x_out(i + 1)
        with jax.named_scope("sa_epilogue"):
            x_out(0)
            for i in range(8):
                o_copy(i).wait()
        return
    acc = jnp.zeros((128, 128), f32)
    for j in range(NJ):
        acc = acc + xT[j, 0:128, :] + xT[j, 896:1024, :] + pbuf[0, j, 0:128, :] + pltpu.bitcast(lhsA[0, 0, 0:8, :], f32)[0:1]
    xraw[0, :, 0:128] = pltpu.bitcast(acc, u32)
    pltpu.sync_copy(xraw.at[0], out_hbm.bitcast(u32).at[:, 0, :])


@jax.jit
def pallas_interleave_layers__linear_kernel_hedgehog__sliding_local_dilated__prompt_kernel(
    A_x, A_wqkv, A_w_phi, A_wo, B_x, B_wqkv, B_wo):
    del B_x
    x2 = A_x.reshape(128, NJ, D)
    hbm = pl.BlockSpec(memory_space=pl.ANY)
    out = pl.pallas_call(
        _kernel,
        out_shape=jax.ShapeDtypeStruct((128, NJ, D), bf16),
        in_specs=[hbm, hbm, pl.BlockSpec(memory_space=pltpu.VMEM), hbm, hbm, hbm],
        out_specs=hbm,
        scratch_shapes=[
            pltpu.VMEM((NJ, D, 128), f32),
            pltpu.VMEM((NJ, D, 128), bf16),
            pltpu.VMEM((2, NG, 8, 384, 128), bf16),
            pltpu.VMEM((2, NG, D, 128), bf16),
            pltpu.VMEM((2, NJ, 384, 128), f32),
            pltpu.VMEM((2, 2, 40, 128), u32),
            pltpu.VMEM((8, 128, D), u32),
            pltpu.VMEM((NG, 7, D, 128), bf16),
            pltpu.VMEM((2, NG, 128, D), bf16),
            pltpu.VMEM((8, 128), u32),
            pltpu.VMEM((2, NJ, 256, 128), f32),
            pltpu.SemaphoreType.DMA((9, 8)),
        ],
        compiler_params=pltpu.CompilerParams(vmem_limit_bytes=100 * 1024 * 1024, flags=FLAGS),
    )(x2, A_wqkv, A_w_phi, A_wo, B_wqkv, B_wo)
    return out.reshape(1, S, D)
```

```python
import jax
import jax.numpy as jnp
import jax.experimental.pallas as pl
import jax.experimental.pallas.tpu as pltpu

f32 = jnp.float32
bf16 = jnp.bfloat16
u32 = jnp.uint32

S, D, H, DH = 2048, 1024, 32, 32
PART = 'ALL'
CFG = 'sm'
FLAGS = None
WC = int('4')
OSPLIT = int('4')
PSK = int('1')
PORD = int('0')
PREPPOS = int('9')
PP = 'ft'
INJ = int('0')
PRESH = int('0')
OFIRST = int('0')
XS = int('3')
XG = int('4')
JIT = int('0')
XJ = int('1')
LSW = int('0')
MG = int('4')
NG = 8
NJ = 16
W, DIL = 8, 2
SCALE = float(DH) ** -0.5
NT = (((1,), (1,)), ((), ()))


NN = (((1,), (0,)), ((), ()))


def _mm(a, b, dims=NN):
    return jax.lax.dot_general(a, b, dims, preferred_element_type=f32)


PW = 1


def _pw(x):
    return x


def _uw(ref):
    return pltpu.bitcast(ref.bitcast(u32)[...], bf16)


def _pk(x):
    return pltpu.bitcast(x, u32)


def _up(x):
    return pltpu.bitcast(x, bf16)


def _recip(x):
    r = pl.reciprocal(x, approx=True)
    return r * (2.0 - x * r)


def _phi(p):
    p3 = p.reshape(4, 32, 128)
    mx = jnp.max(p3, axis=1, keepdims=True)
    mn = jnp.min(p3, axis=1, keepdims=True)
    e1 = jnp.exp(p3 - mx)
    e2 = jnp.exp(mn - p3)
    s1 = jnp.sum(e1, axis=1, keepdims=True)
    s2 = jnp.sum(e2, axis=1, keepdims=True)
    a = (e1 * _recip(s1)).reshape(128, 128)
    b = (e2 * _recip(s2)).reshape(128, 128)
    t0 = jnp.concatenate([a[0:64], b[0:64]], axis=0).astype(bf16)
    t1 = jnp.concatenate([a[64:128], b[64:128]], axis=0).astype(bf16)
    return t0, t1


def _kernel(x_hbm, awqkv_hbm, awphi_ref, awo_hbm, bwqkv_hbm, bwo_hbm, out_hbm,
            xT, lnT, WW, WO, pbuf, lhsA, xraw, wraw, oraw, zref, shbuf, sems):
    zref[...] = jnp.zeros((8, 128), u32)
    full = PART == 'ALL'

    def x_copy(c):
        return pltpu.make_async_copy(x_hbm.bitcast(u32).at[:, c, :], xraw.at[c], sems.at[0, c])

    def col(hbm, part, g):
        return hbm.at[:, pl.ds(pl.multiple_of(part * D + g * 128, 128), 128)]

    def wa_copies(g):
        return [pltpu.make_async_copy(col(awqkv_hbm, p, g), wraw.at[g, p], sems.at[1 + p, g]) for p in range(3)]

    def wb_copies(g):
        return [pltpu.make_async_copy(col(bwqkv_hbm, p, g), wraw.at[g, 4 + p], sems.at[5 + p, g]) for p in range(3)]

    def wo_copies(g):
        rows = pl.ds(pl.multiple_of(g * 128, 128), 128)
        return [pltpu.make_async_copy(awo_hbm.at[rows, :], oraw.at[0, g], sems.at[4, g]),
                pltpu.make_async_copy(bwo_hbm.at[rows, :], oraw.at[1, g], sems.at[8, g])]

    def rest_copies(g):
        return wo_copies(g) + wb_copies(g)

    f_i = jax.lax.broadcasted_iota(jnp.int32, (32, 128), 0)
    c_i = jax.lax.broadcasted_iota(jnp.int32, (32, 128), 1)
    R = jnp.where(c_i % 32 == f_i, 1.0, 0.0).astype(bf16)
    r2 = jax.lax.broadcasted_iota(jnp.int32, (128, 128), 0)
    c2 = jax.lax.broadcasted_iota(jnp.int32, (128, 128), 1)
    blockmask = (r2 // 32) == (c2 // 32)

    def build_w(lt, g):
        tiles = []
        if lt == 0:
            Bm = awphi_ref[pl.ds(4 * g, 4)].reshape(128, 32)
            Phi = jnp.where(blockmask, _mm(Bm, R), 0.0)
            PhiT = Phi.T.astype(bf16)
        for k in range(8):
            ks = slice(k * 128, (k + 1) * 128)
            if lt == 0:
                parts = [_mm(PhiT, wraw[g, 0, ks, :], NT).astype(bf16),
                         _mm(PhiT, wraw[g, 1, ks, :], NT).astype(bf16),
                         wraw[g, 2, ks, :].T]
            else:
                parts = [wraw[g, 4 + p, ks, :].T for p in range(3)]
            t = jnp.concatenate(parts, axis=0)
            WW[lt, g, k] = t
            tiles.append(t)
        return tiles

    def build_wo(lt, g, q, n):
        t = jnp.concatenate([oraw[lt, g, :, c * 128:(c + 1) * 128].T for c in range(q * n // 128, (q + 1) * n // 128)], axis=0)
        WO[lt, g, pl.ds(q * n, n), :] = t
        return t

    def start(cs):
        for c in cs:
            c.start()

    def wait(cs):
        for c in cs:
            c.wait()

    if full:
      with jax.named_scope('s0_prologue'):
        start(wa_copies(0))
        start([x_copy(c) for c in range(8)])
        wait(wa_copies(0))
        build_w(0, 0)

    def x_in(i):
        for c in range(8):
            wd = xraw[i, :, c * 128:(c + 1) * 128].T
            xT[2 * i, c * 128:(c + 1) * 128, :] = pltpu.bitcast(wd << 16, f32)
            xT[2 * i + 1, c * 128:(c + 1) * 128, :] = pltpu.bitcast(wd & jnp.uint32(0xFFFF0000), f32)

    def o_copy(i):
        return pltpu.make_async_copy(xraw.at[i], out_hbm.bitcast(u32).at[:, i, :], sems.at[0, i])

    def x_out(i):
        for c in range(8):
            lo = xT[2 * i, c * 128:(c + 1) * 128, :]
            hi = xT[2 * i + 1, c * 128:(c + 1) * 128, :]
            lo = pltpu.bitcast(lo.astype(bf16).astype(f32), u32) >> 16
            hi = pltpu.bitcast(hi.astype(bf16).astype(f32), u32)
            xraw[i, :, c * 128:(c + 1) * 128] = (lo | hi).T
        o_copy(i).start()

    lane = jax.lax.broadcasted_iota(jnp.int32, (4, 1, 128), 2)
    lane0 = lane == 0
    ones16 = jnp.ones((16, 128), f32)
    odd8 = (jax.lax.broadcasted_iota(jnp.int32, (8, 128), 0) % 2) == 1
    lane0_8 = jax.lax.broadcasted_iota(jnp.int32, (8, 128), 1) == 0
    zero_u = zref[...]

    def ln_step(j):
        x = xT[j]
        m = jnp.sum(x, axis=0, keepdims=True) * (1.0 / D)
        xc = x - m
        v = jnp.sum(xc * xc, axis=0, keepdims=True) * (1.0 / D)
        lnT[j] = (xc * jax.lax.rsqrt(v + 1e-5)).astype(bf16)

    TN = (((0,), (0,)), ((), ()))

    def proj(lt, g, j, build=False):
        if build:
            return _mm(jnp.concatenate(build_w(lt, g), axis=1), _uw(lnT.at[j]))
        if lt == 1 and 'tnp' in CFG:
            return _mm(jnp.concatenate([wraw[g, 4 + p] for p in range(3)], axis=1), lnT[j], TN)
        return _mm(jnp.concatenate([_uw(WW.at[lt, g, k]) for k in range(8)], axis=1), _uw(lnT.at[j]))

    def out_proj(lt, g, j, o, build=False):
        n = 1024 // OSPLIT
        for q in range(OSPLIT):
            if build:
                xT[j, q * n:(q + 1) * n, :] += _mm(build_wo(lt, g, q, n), o)
                continue
            if 'tno' in CFG:
                xT[j, q * n:(q + 1) * n, :] += _mm(oraw[lt, g, :, q * n:(q + 1) * n], o, TN)
                continue
            xT[j, q * n:(q + 1) * n, :] += _mm(_uw(WO.at[lt, g, pl.ds(q * n, n)]), o)

    def kv_step(pk, v, acc):
        t0, t1 = _phi(pk)
        l0 = jnp.concatenate([v[0:64], ones16], axis=0).astype(bf16)
        l1 = jnp.concatenate([v[64:128], ones16], axis=0).astype(bf16)
        a0 = _mm(l0, t0, NT)
        a1 = _mm(l1, t1, NT)
        if acc is None:
            return a0, a1
        return acc[0] + a0, acc[1] + a1

    rr = jax.lax.broadcasted_iota(jnp.int32, (80, 128), 0)
    cc = jax.lax.broadcasted_iota(jnp.int32, (80, 128), 1)
    row_head = jnp.where(rr < 64, rr // 32, (rr - 64) // 8)
    kvmask = row_head == ((cc // 32) % 2)

    def kv_final(acc, slot):
        lhsA[slot, 0] = _pk(jnp.where(kvmask, acc[0], 0.0).astype(bf16))
        lhsA[slot, 1] = _pk(jnp.where(kvmask, acc[1], 0.0).astype(bf16))

    def num_step(pq, slot, deps=()):
        t0, t1 = _phi(pq)
        outs = []
        for p, t in ((0, t0), (1, t1)):
            lw = lhsA[slot, p]
            if p == 0:
                z = None
                for dv in deps:
                    if dv is not None:
                        z = dv[56:64, :] if z is None else z | dv[56:64, :]
                if z is not None:
                    lw = jnp.concatenate([lw[0:8] | (z & zero_u), lw[8:]], axis=0)
            r = _mm(_up(lw), t)
            for hh in range(2):
                den = r[64 + 8 * hh: 72 + 8 * hh] + 1e-6
                num = r[32 * hh: 32 * hh + 32].reshape(4, 8, 128)
                outs.append((num * _recip(den)[None]).reshape(32, 128))
        return jnp.concatenate(outs, axis=0).astype(bf16)

    def att_tile(slot, j, kcache, vcache):
        def get(cache, base, jj):
            if jj not in cache:
                if jj >= 0:
                    cache[jj] = pbuf[slot, jj, base:base + 128, :]
                else:
                    if PRESH:
                        cache[jj] = shbuf[slot, jj + 16, base - 128:base, :]
                    else:
                        cache[jj] = pltpu.roll(pbuf[slot, jj + 16, base:base + 128, :], 1, 1)
            return cache[jj]
        def one(h0, nh, dep):
            rows = lambda base: slice(base + 32 * h0, base + 32 * (h0 + nh))
            q = pbuf[slot, j, rows(0), :].reshape(nh, 32, 128)
            if dep is not None:
                q = q + dep
            ls = []
            for w in range(W):
                jj = j - DIL * w
                kk = get(kcache, 128, jj)[32 * h0: 32 * (h0 + nh)].reshape(nh, 32, 128)
                if 'wchain' in CFG and w > 0 and w % WC == 0:
                    qq = q + ls[-1][0:1] * 0.0
                else:
                    qq = q
                l = jnp.sum(qq * kk, axis=1, keepdims=True) * SCALE
                if jj < 0:
                    l = jnp.where(lane0[:nh], -1e9, l)
                ls.append(l)
            m = ls[0]
            for w in range(1, W):
                m = jnp.maximum(m, ls[w])
            es = [jnp.exp(l - m) for l in ls]
            ssum = es[0]
            for w in range(1, W):
                ssum = ssum + es[w]
            r = _recip(ssum)
            o = None
            for w in range(W):
                vv = get(vcache, 256, j - DIL * w)[32 * h0: 32 * (h0 + nh)].reshape(nh, 32, 128)
                t = (es[w] * r) * vv
                o = t if o is None else o + t
            return o
        if 'sm' in CFG:
            q = pbuf[slot, j, 0:128, :].reshape(16, 8, 128)
            ls = []
            for w in range(W):
                jj = j - DIL * w
                kk = get(kcache, 128, jj).reshape(16, 8, 128)
                a = jnp.sum(q * kk, axis=0)
                l = (a + pltpu.roll(a, 4, 0)) * SCALE
                if jj < 0:
                    l = jnp.where(lane0_8, -1e9, l)
                ls.append(l)
            m = ls[0]
            for w in range(1, W):
                m = jnp.maximum(m, ls[w])
            es = [jnp.exp(l - m) for l in ls]
            ssum = es[0]
            for w in range(1, W):
                ssum = ssum + es[w]
            r = _recip(ssum)
            if 'smv' in CFG:
                o = None
                for w in range(W):
                    vv = get(vcache, 256, j - DIL * w).reshape(16, 8, 128)
                    t = (es[w] * r)[None] * vv
                    o = t if o is None else o + t
                return o.reshape(128, 128).astype(bf16)
            outs = []
            aw = [es[w] * r for w in range(W)]
            for hh in range(4):
                o = None
                for w in range(W):
                    vv = get(vcache, 256, j - DIL * w)[32 * hh:32 * hh + 32].reshape(4, 8, 128)
                    t = aw[w][hh:hh + 1][None] * vv
                    o = t if o is None else o + t
                outs.append(o.reshape(32, 128))
            return jnp.concatenate(outs, axis=0).astype(bf16)
        if 'dm' in CFG:
            q = pbuf[slot, j, 0:128, :].reshape(16, 8, 128)
            ls = []
            for w in range(W):
                jj = j - DIL * w
                kk = get(kcache, 128, jj).reshape(16, 8, 128)
                a = jnp.sum(q * kk, axis=0)
                l = (a + jnp.where(odd8, pltpu.roll(a, 1, 0), pltpu.roll(a, 7, 0))) * SCALE
                if jj < 0:
                    l = jnp.where(lane0_8, -1e9, l)
                ls.append(l)
            m = ls[0]
            for w in range(1, W):
                m = jnp.maximum(m, ls[w])
            es = [jnp.exp(l - m) for l in ls]
            ssum = es[0]
            for w in range(1, W):
                ssum = ssum + es[w]
            r = _recip(ssum)
            o = None
            for w in range(W):
                vv = get(vcache, 256, j - DIL * w).reshape(16, 8, 128)
                t = (es[w] * r)[None] * vv
                o = t if o is None else o + t
            return o.reshape(128, 128).astype(bf16)
        if 'chain' in CFG:
            nh = 2 if 'chain2' in CFG else 1
            outs = []
            dep = None
            for h0 in range(0, 4, nh):
                o = one(h0, nh, dep)
                dep = o[0:1, 0:1, :] * 0.0
                outs.append(o.reshape(32 * nh, 128))
            return jnp.concatenate(outs, axis=0).astype(bf16)
        return one(0, 4, None).reshape(128, 128).astype(bf16)

    def block(front, back, ln, prep=None, bw=False, bo=False, js=None, st0=None, fin=True, xin=False, nb=None):
        st = st0 if st0 is not None else {'acc': None, 'p1': False, 'o1': False}
        pend, ots = {}, {}
        kc, vc = st.setdefault('kc', {}), st.setdefault('vc', {})
        ft = front[0] if front else None
        bt = back[0] if back else None
        order = list(range(NJ - 1, -1, -1)) if bt == 'B' else list(range(NJ))

        def P(j):
            _, g, slot = front
            if xin and j % 2 == 0:
                x_in(j // 2)
            if ln:
                ln_step(j)
            r = proj(0 if ft == 'A' else 1, g, j, bw and not st['p1'])
            st['p1'] = True
            if ft == 'A':
                pbuf[slot, j, 0:128, :] = r[0:128]
                pend[j] = (r[128:256], r[256:384])
            else:
                if 'sm' in CFG:
                    np_ = 3 if 'smv' in CFG else 2
                    for part in range(np_):
                        for hh in range(4):
                            for a in range(4):
                                r0 = part * 128 + hh * 32 + a * 8
                                pbuf.at[slot, j][pl.ds(part * 128 + 32 * a + hh, 8, stride=4), :] = r[r0:r0 + 8]
                    if np_ == 2:
                        pbuf[slot, j, 256:384, :] = r[256:384]
                else:
                    pbuf[slot, j, 0:384, :] = r
                if PRESH and j >= DIL:
                    shbuf[slot, j, 0:128, :] = pltpu.roll(r[128:256], 1, 1)
                    shbuf[slot, j, 128:256, :] = pltpu.roll(r[256:384], 1, 1)

        def KV(j):
            pk, v = pend.pop(j)
            st['acc'] = kv_step(pk, v, st['acc'])

        def NUM(j):
            _, g, slot = back
            ots[j] = num_step(pbuf[slot, j, 0:128, :], slot)

        def O(j):
            _, g, slot = back
            if bt == 'A':
                out_proj(0, g, j, ots.pop(j), bo and not st['o1'])
                st['o1'] = True
            else:
                out_proj(1, g, j, att_tile(slot, j, kc, vc), bo and not st['o1'])
            st['o1'] = True

        if js is not None:
            order = list(js)
        n = len(order)
        nbk = n if nb is None else nb
        psk = PSK if (ln and back) else 0
        for t in range(-1, n + psk + 2):
            if bt == 'A' and 0 <= t + 1 < nbk:
                NUM(order[t + 1])
            of = psk or OFIRST or (t >= n - LSW)
            if of and back and 0 <= t < nbk:
                O(order[t])
            if front and 0 <= t - psk < n:
                P((order if ln or PORD or js is not None else list(range(NJ)))[t - psk])
            if not of and back and 0 <= t < nbk:
                O(order[t])
            if ft == 'A' and 0 <= t - psk - 1 < n:
                KV(order[t - psk - 1])
        if ft == 'A' and fin:
            kv_final(st['acc'], front[2])
        if prep is not None:
            prep()

    def prep_next(g, gn):
        if gn is not None:
            build_w(0, gn)
        if not (JIT & 1):
            build_wo(0, g, 0, 1024)
        if not (JIT & 2):
            build_w(1, g)
        if not (JIT & 4):
            build_wo(1, g, 0, 1024)

    def a_loop(first):
        def body(g, _):
            slot = g % 2
            prep = None
            if first:
                @pl.when(g + 1 < NG)
                def _():
                    wait(wa_copies(g + 1))
                    start(rest_copies(g + 1))

                @pl.when(g + 2 < NG)
                def _():
                    start(wa_copies(g + 2))
                wait(rest_copies(g))
                prep = lambda: prep_next(g, jnp.minimum(g + 1, NG - 1))
            block(('A', g, slot), ('A', g - 1, 1 - slot), False, prep, bo=first and bool(JIT & 1))
            return 0
        jax.lax.fori_loop(1, NG - (1 if MG else 0), body, 0)

    def b_loop(first):
        def body(g, _):
            slot = g % 2
            block(('B', g, slot), ('B', g - 1, 1 - slot), False, bw=first and bool(JIT & 2), bo=first and bool(JIT & 4))
            return 0
        jax.lax.fori_loop(1, NG - (1 if MG else 0), body, 0)

    L = (NG - 1) % 2

    def tail(bt, js):
        block(None, (bt, NG - 2, 1 - L), False, js=js)

    def trans(ft, bt, prep=None):
        if MG:
            order = list(range(NJ - 1, -1, -1)) if bt == 'B' else list(range(NJ))
            block((bt, NG - 1, L), (bt, NG - 2, 1 - L), False, prep, nb=NJ - MG)
            tail(bt, order[NJ - MG:])
        block((ft, 0, 0) if ft else None, (bt, NG - 1, L), True if ft else False)

    if PART == 'A':
        a_loop(False)
    elif PART == 'A1':
        a_loop(True)
    elif PART == 'B':
        b_loop(False)
    elif PART == 'B1':
        b_loop(True)
    elif PART == 'BS':
        block(('B', 1, 0), ('B', 0, 1), False)
    elif PART == 'AS':
        block(('A', 1, 0), ('A', 0, 1), False)
    elif PART == 'AB':
        trans('B', 'A')
    elif PART == 'BA':
        trans('A', 'B')
    elif PART == 'INIT':
        block(('A', 0, 0), None, True)
    elif PART == 'FIN':
        block(None, ('B', NG - 1, L), False)
    else:
        sti = {'acc': None, 'p1': False, 'o1': False}
        for h in range(8 // XG):
            with jax.named_scope("s1_init"):
                for i in range(h * XG, (h + 1) * XG):
                    x_copy(i).wait()
                    if not XJ:
                        x_in(i)
                    if i == XS:
                        start(wa_copies(1) + rest_copies(0))
            with jax.named_scope("s1_initb"):
                last = h == 8 // XG - 1
                if last:
                    start(wa_copies(2) + rest_copies(1))

                def prep0():
                    wait(wa_copies(1) + rest_copies(0))
                    prep_next(0, 1)
                block(('A', 0, 0), None, True, prep0 if last else None, js=range(2 * XG * h, 2 * XG * (h + 1)), st0=sti, fin=last, xin=bool(XJ))
        with jax.named_scope("s2_loopA1"):
            a_loop(True)
        with jax.named_scope("s3_AB"):
            if MG:
                wait(rest_copies(NG - 1))
            trans('B', 'A', (lambda: prep_next(NG - 1, None)) if MG else None)
        with jax.named_scope("s4_loopB1"):
            b_loop(True)
        with jax.named_scope("s5_BA"):
            trans('A', 'B')
        with jax.named_scope("s6_loopA2"):
            a_loop(False)
        with jax.named_scope("s7_AB"):
            trans('B', 'A')
        with jax.named_scope("s8_loopB"):
            b_loop(False)
        stf = {'acc': None, 'p1': False, 'o1': False}
        if MG:
            with jax.named_scope("s8_last"):
                block(('B', NG - 1, L), ('B', NG - 2, 1 - L), False, nb=NJ - MG)
                tail('B', list(range(NJ - 1, -1, -1))[NJ - MG:])
                block(None, ('B', NG - 1, L), False, js=(15, 14), st0=stf)
        for i in range(7, -1, -1):
            with jax.named_scope("s9_fin"):
                if not (MG and i == 7):
                    block(None, ('B', NG - 1, L), False, js=(2 * i + 1, 2 * i), st0=stf)
                if i < 7:
                    x_out(i + 1)
        with jax.named_scope("sa_epilogue"):
            x_out(0)
            for i in range(8):
                o_copy(i).wait()
        return
    acc = jnp.zeros((128, 128), f32)
    for j in range(NJ):
        acc = acc + xT[j, 0:128, :] + xT[j, 896:1024, :] + pbuf[0, j, 0:128, :] + pltpu.bitcast(lhsA[0, 0, 0:8, :], f32)[0:1]
    xraw[0, :, 0:128] = pltpu.bitcast(acc, u32)
    pltpu.sync_copy(xraw.at[0], out_hbm.bitcast(u32).at[:, 0, :])


@jax.jit
def pallas_interleave_layers__linear_kernel_hedgehog__sliding_local_dilated__prompt_kernel(
    A_x, A_wqkv, A_w_phi, A_wo, B_x, B_wqkv, B_wo):
    del B_x
    x2 = A_x.reshape(128, NJ, D)
    hbm = pl.BlockSpec(memory_space=pl.ANY)
    out = pl.pallas_call(
        _kernel,
        out_shape=jax.ShapeDtypeStruct((128, NJ, D), bf16),
        in_specs=[hbm, hbm, pl.BlockSpec(memory_space=pltpu.VMEM), hbm, hbm, hbm],
        out_specs=hbm,
        scratch_shapes=[
            pltpu.VMEM((NJ, D, 128), f32),
            pltpu.VMEM((NJ, D, 128), bf16),
            pltpu.VMEM((2, NG, 8, 384, 128), bf16),
            pltpu.VMEM((2, NG, D, 128), bf16),
            pltpu.VMEM((2, NJ, 384, 128), f32),
            pltpu.VMEM((2, 2, 40, 128), u32),
            pltpu.VMEM((8, 128, D), u32),
            pltpu.VMEM((NG, 7, D, 128), bf16),
            pltpu.VMEM((2, NG, 128, D), bf16),
            pltpu.VMEM((8, 128), u32),
            pltpu.VMEM((2, NJ, 256, 128), f32),
            pltpu.SemaphoreType.DMA((9, 8)),
        ],
        compiler_params=pltpu.CompilerParams(vmem_limit_bytes=100 * 1024 * 1024, flags=FLAGS),
    )(x2, A_wqkv, A_w_phi, A_wo, B_wqkv, B_wo)
    return out.reshape(1, S, D)
```

```python
import jax
import jax.numpy as jnp
import jax.experimental.pallas as pl
import jax.experimental.pallas.tpu as pltpu

f32 = jnp.float32
bf16 = jnp.bfloat16
u32 = jnp.uint32

S, D, H, DH = 2048, 1024, 32, 32
OSPLIT = 4
MG = 4
XS = 7
NG = 8
NJ = 16
W, DIL = 8, 2
SCALE = float(DH) ** -0.5
NT = (((1,), (1,)), ((), ()))


NN = (((1,), (0,)), ((), ()))


def _mm(a, b, dims=NN):
    return jax.lax.dot_general(a, b, dims, preferred_element_type=f32)


PW = 1


def _pw(x):
    return x


def _uw(ref):
    return pltpu.bitcast(ref.bitcast(u32)[...], bf16)


def _pk(x):
    return pltpu.bitcast(x, u32)


def _up(x):
    return pltpu.bitcast(x, bf16)


def _recip(x):
    r = pl.reciprocal(x, approx=True)
    return r * (2.0 - x * r)


def _phi(p):
    p3 = p.reshape(4, 32, 128)
    mx = jnp.max(p3, axis=1, keepdims=True)
    mn = jnp.min(p3, axis=1, keepdims=True)
    e1 = jnp.exp(p3 - mx)
    e2 = jnp.exp(mn - p3)
    s1 = jnp.sum(e1, axis=1, keepdims=True)
    s2 = jnp.sum(e2, axis=1, keepdims=True)
    a = (e1 * _recip(s1)).reshape(128, 128)
    b = (e2 * _recip(s2)).reshape(128, 128)
    t0 = jnp.concatenate([a[0:64], b[0:64]], axis=0).astype(bf16)
    t1 = jnp.concatenate([a[64:128], b[64:128]], axis=0).astype(bf16)
    return t0, t1


def _kernel(x_hbm, awqkv_hbm, awphi_ref, awo_hbm, bwqkv_hbm, bwo_hbm, out_hbm,
            xT, lnT, WW, WO, pbuf, lhsA, xraw, wraw, oraw, sems):

    def x_copy(c):
        return pltpu.make_async_copy(x_hbm.bitcast(u32).at[:, c, :], xraw.at[c], sems.at[0, c])

    def col(hbm, part, g):
        return hbm.at[:, pl.ds(pl.multiple_of(part * D + g * 128, 128), 128)]

    def wa_copies(g):
        return [pltpu.make_async_copy(col(awqkv_hbm, p, g), wraw.at[g, p], sems.at[1 + p, g]) for p in range(3)]

    def wb_copies(g):
        return [pltpu.make_async_copy(col(bwqkv_hbm, p, g), wraw.at[g, 4 + p], sems.at[5 + p, g]) for p in range(3)]

    def wo_copies(g):
        rows = pl.ds(pl.multiple_of(g * 128, 128), 128)
        return [pltpu.make_async_copy(awo_hbm.at[rows, :], oraw.at[0, g], sems.at[4, g]),
                pltpu.make_async_copy(bwo_hbm.at[rows, :], oraw.at[1, g], sems.at[8, g])]

    def rest_copies(g):
        return wo_copies(g) + wb_copies(g)

    f_i = jax.lax.broadcasted_iota(jnp.int32, (32, 128), 0)
    c_i = jax.lax.broadcasted_iota(jnp.int32, (32, 128), 1)
    R = jnp.where(c_i % 32 == f_i, 1.0, 0.0).astype(bf16)
    r2 = jax.lax.broadcasted_iota(jnp.int32, (128, 128), 0)
    c2 = jax.lax.broadcasted_iota(jnp.int32, (128, 128), 1)
    blockmask = (r2 // 32) == (c2 // 32)

    def build_w(lt, g):
        tiles = []
        if lt == 0:
            Bm = awphi_ref[pl.ds(4 * g, 4)].reshape(128, 32)
            Phi = jnp.where(blockmask, _mm(Bm, R), 0.0)
            PhiT = Phi.T.astype(bf16)
        for k in range(8):
            ks = slice(k * 128, (k + 1) * 128)
            if lt == 0:
                parts = [_mm(PhiT, wraw[g, 0, ks, :], NT).astype(bf16),
                         _mm(PhiT, wraw[g, 1, ks, :], NT).astype(bf16),
                         wraw[g, 2, ks, :].T]
            else:
                parts = [wraw[g, 4 + p, ks, :].T for p in range(3)]
            t = jnp.concatenate(parts, axis=0)
            WW[lt, g, k] = t
            tiles.append(t)
        return tiles

    def build_wo(lt, g, q, n):
        t = jnp.concatenate([oraw[lt, g, :, c * 128:(c + 1) * 128].T for c in range(q * n // 128, (q + 1) * n // 128)], axis=0)
        WO[lt, g, pl.ds(q * n, n), :] = t
        return t

    def start(cs):
        for c in cs:
            c.start()

    def wait(cs):
        for c in cs:
            c.wait()

    with jax.named_scope('s0_prologue'):
        start(wa_copies(0))
        start([x_copy(c) for c in range(8)])
        wait(wa_copies(0))
        build_w(0, 0)

    def x_in(i):
        for c in range(8):
            wd = xraw[i, :, c * 128:(c + 1) * 128].T
            xT[2 * i, c * 128:(c + 1) * 128, :] = pltpu.bitcast(wd << 16, f32)
            xT[2 * i + 1, c * 128:(c + 1) * 128, :] = pltpu.bitcast(wd & jnp.uint32(0xFFFF0000), f32)

    def o_copy(i):
        return pltpu.make_async_copy(xraw.at[i], out_hbm.bitcast(u32).at[:, i, :], sems.at[0, i])

    def x_out(i):
        for c in range(8):
            lo = xT[2 * i, c * 128:(c + 1) * 128, :]
            hi = xT[2 * i + 1, c * 128:(c + 1) * 128, :]
            lo = pltpu.bitcast(lo.astype(bf16).astype(f32), u32) >> 16
            hi = pltpu.bitcast(hi.astype(bf16).astype(f32), u32)
            xraw[i, :, c * 128:(c + 1) * 128] = (lo | hi).T
        o_copy(i).start()

    lane = jax.lax.broadcasted_iota(jnp.int32, (4, 1, 128), 2)
    lane0 = lane == 0
    ones16 = jnp.ones((16, 128), f32)
    odd8 = (jax.lax.broadcasted_iota(jnp.int32, (8, 128), 0) % 2) == 1
    lane0_8 = jax.lax.broadcasted_iota(jnp.int32, (8, 128), 1) == 0

    def ln_step(j):
        x = xT[j]
        m = jnp.sum(x, axis=0, keepdims=True) * (1.0 / D)
        xc = x - m
        v = jnp.sum(xc * xc, axis=0, keepdims=True) * (1.0 / D)
        lnT[j] = (xc * jax.lax.rsqrt(v + 1e-5)).astype(bf16)

    TN = (((0,), (0,)), ((), ()))

    def proj(lt, g, j, build=False):
        return _mm(jnp.concatenate([_uw(WW.at[lt, g, k]) for k in range(8)], axis=1), _uw(lnT.at[j]))

    def out_proj(lt, g, j, o, build=False):
        n = 1024 // OSPLIT
        for q in range(OSPLIT):
            xT[j, q * n:(q + 1) * n, :] += _mm(_uw(WO.at[lt, g, pl.ds(q * n, n)]), o)

    def kv_step(pk, v, acc):
        t0, t1 = _phi(pk)
        l0 = jnp.concatenate([v[0:64], ones16], axis=0).astype(bf16)
        l1 = jnp.concatenate([v[64:128], ones16], axis=0).astype(bf16)
        a0 = _mm(l0, t0, NT)
        a1 = _mm(l1, t1, NT)
        if acc is None:
            return a0, a1
        return acc[0] + a0, acc[1] + a1

    rr = jax.lax.broadcasted_iota(jnp.int32, (80, 128), 0)
    cc = jax.lax.broadcasted_iota(jnp.int32, (80, 128), 1)
    row_head = jnp.where(rr < 64, rr // 32, (rr - 64) // 8)
    kvmask = row_head == ((cc // 32) % 2)

    def kv_final(acc, slot):
        lhsA[slot, 0] = _pk(jnp.where(kvmask, acc[0], 0.0).astype(bf16))
        lhsA[slot, 1] = _pk(jnp.where(kvmask, acc[1], 0.0).astype(bf16))

    def num_step(pq, slot, deps=()):
        t0, t1 = _phi(pq)
        outs = []
        for p, t in ((0, t0), (1, t1)):
            lw = lhsA[slot, p]
            if p == 0:
                z = None
                for dv in deps:
                    if dv is not None:
                        z = dv[56:64, :] if z is None else z | dv[56:64, :]
                if z is not None:
                    lw = jnp.concatenate([lw[0:8] | (z & zero_u), lw[8:]], axis=0)
            r = _mm(_up(lw), t)
            for hh in range(2):
                den = r[64 + 8 * hh: 72 + 8 * hh] + 1e-6
                num = r[32 * hh: 32 * hh + 32].reshape(4, 8, 128)
                outs.append((num * _recip(den)[None]).reshape(32, 128))
        return jnp.concatenate(outs, axis=0).astype(bf16)

    def att_tile(slot, j, kcache, vcache):
        def get(cache, base, jj):
            if jj not in cache:
                if jj >= 0:
                    cache[jj] = pbuf[slot, jj, base:base + 128, :]
                else:
                    cache[jj] = pltpu.roll(pbuf[slot, jj + 16, base:base + 128, :], 1, 1)
            return cache[jj]
        if True:
            q = pbuf[slot, j, 0:128, :].reshape(16, 8, 128)
            ls = []
            for w in range(W):
                jj = j - DIL * w
                kk = get(kcache, 128, jj).reshape(16, 8, 128)
                a = jnp.sum(q * kk, axis=0)
                l = (a + pltpu.roll(a, 4, 0)) * SCALE
                if jj < 0:
                    l = jnp.where(lane0_8, -1e9, l)
                ls.append(l)
            m = ls[0]
            for w in range(1, W):
                m = jnp.maximum(m, ls[w])
            es = [jnp.exp(l - m) for l in ls]
            ssum = es[0]
            for w in range(1, W):
                ssum = ssum + es[w]
            r = _recip(ssum)
            outs = []
            aw = [es[w] * r for w in range(W)]
            for hh in range(4):
                o = None
                for w in range(W):
                    vv = get(vcache, 256, j - DIL * w)[32 * hh:32 * hh + 32].reshape(4, 8, 128)
                    t = aw[w][hh:hh + 1][None] * vv
                    o = t if o is None else o + t
                outs.append(o.reshape(32, 128))
            return jnp.concatenate(outs, axis=0).astype(bf16)
    def block(front, back, ln, prep=None, bw=False, bo=False, js=None, st0=None, fin=True, xin=False, nb=None, mid=()):
        st = st0 if st0 is not None else {'acc': None, 'p1': False, 'o1': False}
        pend, ots = {}, {}
        kc, vc = st.setdefault('kc', {}), st.setdefault('vc', {})
        ft = front[0] if front else None
        bt = back[0] if back else None
        order = list(range(NJ - 1, -1, -1)) if bt == 'B' else list(range(NJ))

        def P(j):
            _, g, slot = front
            if xin and j % 2 == 0:
                x_in(j // 2)
            if ln:
                ln_step(j)
            r = proj(0 if ft == 'A' else 1, g, j, bw and not st['p1'])
            st['p1'] = True
            if ft == 'A':
                pbuf[slot, j, 0:128, :] = r[0:128]
                pend[j] = (r[128:256], r[256:384])
            else:
                for part in range(2):
                    for hh in range(4):
                        for a in range(4):
                            r0 = part * 128 + hh * 32 + a * 8
                            pbuf.at[slot, j][pl.ds(part * 128 + 32 * a + hh, 8, stride=4), :] = r[r0:r0 + 8]
                pbuf[slot, j, 256:384, :] = r[256:384]

        def KV(j):
            pk, v = pend.pop(j)
            st['acc'] = kv_step(pk, v, st['acc'])

        def NUM(j):
            _, g, slot = back
            ots[j] = num_step(pbuf[slot, j, 0:128, :], slot)

        def O(j):
            _, g, slot = back
            if bt == 'A':
                out_proj(0, g, j, ots.pop(j), bo and not st['o1'])
                st['o1'] = True
            else:
                out_proj(1, g, j, att_tile(slot, j, kc, vc), bo and not st['o1'])
            st['o1'] = True

        if js is not None:
            order = list(js)
        n = len(order)
        nbk = n if nb is None else nb
        psk = 1 if (ln and back) else 0
        for t in range(-1, n + psk + 1 + 1):
            if bt == 'A' and 0 <= t + 1 < nbk:
                NUM(order[t + 1])
            of = psk
            if of and back and 0 <= t < nbk:
                O(order[t])
            if front and 0 <= t - psk < n:
                P((order if ln or js is not None else list(range(NJ)))[t - psk])
            if not of and back and 0 <= t < nbk:
                O(order[t])
            if 0 <= t < len(mid):
                mid[t]()
            if ft == 'A' and 0 <= t - psk - 1 < n:
                KV(order[t - psk - 1])
        if ft == 'A' and fin:
            kv_final(st['acc'], front[2])
        if prep is not None:
            prep()

    def prep_next(g, gn):
        if gn is not None:
            build_w(0, gn)
        build_wo(0, g, 0, 1024)
        build_w(1, g)
        build_wo(1, g, 0, 1024)

    def a_loop(first):
        def body(g, _):
            slot = g % 2
            prep = None
            if first:
                @pl.when(g + 1 < NG)
                def _():
                    wait(wa_copies(g + 1))
                    start(rest_copies(g + 1))

                @pl.when(g + 2 < NG)
                def _():
                    start(wa_copies(g + 2))
                wait(rest_copies(g))
                prep = lambda: prep_next(g, g + 1)
            block(('A', g, slot), ('A', g - 1, 1 - slot), False, prep)
            return 0
        jax.lax.fori_loop(1, NG - (1 if MG else 0), body, 0)

    def b_loop(first):
        def body(g, _):
            slot = g % 2
            block(('B', g, slot), ('B', g - 1, 1 - slot), False)
            return 0
        jax.lax.fori_loop(1, NG - (1 if MG else 0), body, 0)

    L = (NG - 1) % 2

    def tail(bt, js):
        block(None, (bt, NG - 2, 1 - L), False, js=js)

    def trans(ft, bt, prep=None):
        if MG:
            order = list(range(NJ - 1, -1, -1)) if bt == 'B' else list(range(NJ))
            block((bt, NG - 1, L), (bt, NG - 2, 1 - L), False, prep, nb=NJ - MG)
            tail(bt, order[NJ - MG:])
        block((ft, 0, 0) if ft else None, (bt, NG - 1, L), True if ft else False)

    sti = {'acc': None, 'p1': False, 'o1': False}
    bounds = [0] + [3] + [8]
    for h in range(len(bounds) - 1):
        last = h == len(bounds) - 2
        with jax.named_scope("s1_init"):
            for i in range(bounds[h], bounds[h + 1]):
                x_copy(i).wait()
                if i == XS:
                    start(wa_copies(1) + rest_copies(0))
        with jax.named_scope("s1_initb"):
            if last:
                start(wa_copies(2) + rest_copies(1))

            def prep0():
                wait(wa_copies(1) + rest_copies(0))
                prep_next(0, 1)
            block(('A', 0, 0), None, True, prep0 if last else None, js=range(2 * bounds[h], 2 * bounds[h + 1]), st0=sti, fin=last, xin=True)
    with jax.named_scope("s2_loopA1"):
        a_loop(True)
    with jax.named_scope("s3_AB"):
        if MG:
            wait(rest_copies(NG - 1))
        trans('B', 'A', (lambda: prep_next(NG - 1, None)) if MG else None)
    with jax.named_scope("s4_loopB1"):
        b_loop(True)
    with jax.named_scope("s5_BA"):
        trans('A', 'B')
    with jax.named_scope("s6_loopA2"):
        a_loop(False)
    with jax.named_scope("s7_AB"):
        trans('B', 'A')
    with jax.named_scope("s8_loopB"):
        b_loop(False)
    stf = {'acc': None, 'p1': False, 'o1': False}
    if MG:
        with jax.named_scope("s8_last"):
            block(('B', NG - 1, L), ('B', NG - 2, 1 - L), False, nb=NJ - MG)
            tail('B', list(range(NJ - 1, -1, -1))[NJ - MG:])
            block(None, ('B', NG - 1, L), False, js=(15, 14), st0=stf)
    done = []
    todo = [7]
    for grp in [[6], [5], [4], [3], [2], [1], [0]]:
        with jax.named_scope("s9_fin"):
            for i in grp:
                block(None, ('B', NG - 1, L), False, js=(2 * i + 1, 2 * i), st0=stf)
            for i in todo:
                x_out(i)
            todo = list(grp)
    with jax.named_scope("sa_epilogue"):
        for i in todo:
            x_out(i)
        for i in range(8):
            o_copy(i).wait()


@jax.jit
def pallas_interleave_layers__linear_kernel_hedgehog__sliding_local_dilated__prompt_kernel(
    A_x, A_wqkv, A_w_phi, A_wo, B_x, B_wqkv, B_wo):
    del B_x
    x2 = A_x.reshape(128, NJ, D)
    hbm = pl.BlockSpec(memory_space=pl.ANY)
    out = pl.pallas_call(
        _kernel,
        out_shape=jax.ShapeDtypeStruct((128, NJ, D), bf16),
        in_specs=[hbm, hbm, pl.BlockSpec(memory_space=pltpu.VMEM), hbm, hbm, hbm],
        out_specs=hbm,
        scratch_shapes=[
            pltpu.VMEM((NJ, D, 128), f32),
            pltpu.VMEM((NJ, D, 128), bf16),
            pltpu.VMEM((2, NG, 8, 384, 128), bf16),
            pltpu.VMEM((2, NG, D, 128), bf16),
            pltpu.VMEM((2, NJ, 384, 128), f32),
            pltpu.VMEM((2, 2, 40, 128), u32),
            pltpu.VMEM((8, 128, D), u32),
            pltpu.VMEM((NG, 7, D, 128), bf16),
            pltpu.VMEM((2, NG, 128, D), bf16),
            pltpu.SemaphoreType.DMA((9, 8)),
        ],
        compiler_params=pltpu.CompilerParams(vmem_limit_bytes=100 * 1024 * 1024),
    )(x2, A_wqkv, A_w_phi, A_wo, B_wqkv, B_wo)
    return out.reshape(1, S, D)
```
